```python
import jax
import jax.numpy as jnp

def _softmax(x, axis=-1):
    return jax.nn.softmax(x, axis=axis)

def _gelu(x):
    return jax.nn.gelu(x, approximate=True)

def _silu(x):
    return jax.nn.silu(x)

def _sigmoid(x):
    return jax.nn.sigmoid(x)

def _layernorm(x, axis=-1, eps=1e-05):
    m = jnp.mean(x, axis=axis, keepdims=True)
    v = jnp.var(x, axis=axis, keepdims=True)
    return (x - m) / jnp.sqrt(v + eps)

def _scatter_add(tgt, idx, src, axis=0):
    return tgt.at[idx].add(src)

def _segment_sum(src, seg, n):
    return jax.ops.segment_sum(src, seg, n)

class _Rng:

    def __init__(self, key):
        self._k = key

    def _next(self):
        self._k, sub = jax.random.split(self._k)
        return sub

    def normal(self, shape):
        return jax.random.normal(self._next(), shape, dtype=jnp.bfloat16)

    def randint(self, lo, hi, shape):
        return jax.random.randint(self._next(), shape, lo, hi, dtype=jnp.int32)

    def uniform(self, shape, lo=0.0, hi=1.0):
        return jax.random.uniform(self._next(), shape, jnp.bfloat16, lo, hi)

    def permutation(self, n):
        return jax.random.permutation(self._next(), n)
kernel_name = 'adaLN_cond__sliding_block_cached__moe_arch_mod__decode'

def setup_inputs():
    _rng = _Rng(jax.random.key(int.from_bytes(__import__("os").urandom(4), "little")))
    _w = lambda a: (lambda t: t.astype(jnp.bfloat16) if jnp.issubdtype(t.dtype, jnp.floating) else t)(jnp.asarray(a))

    def _A_setup():
        B, Sq, D = (8, 1, 576)
        Hq, Hkv, Sk, Dh = (32, 16, 8192, 128)
        assert Hq % Hkv == 0, (Hq, Hkv)
        return {'x': _w((lambda *s: _rng.normal(s) * 0.05)(B, Sq, D)), 'k_cache': _w((lambda *s: _rng.normal(s) * 0.05)(B, Hkv, Sk, Dh)), 'v_cache': _w((lambda *s: _rng.normal(s) * 0.05)(B, Hkv, Sk, Dh)), 'wq': _w((lambda *s: _rng.normal(s) * 0.05)(D, Hq * Dh) * D ** (-0.5)), 'wo': _w((lambda *s: _rng.normal(s) * 0.05)(Hq * Dh, D) * (Hq * Dh) ** (-0.5))}
    _A_in = _A_setup()

    def _B_setup():
        B, S, D, F, C = (8, 1, 576, 4608, 1)
        return {'x': _w((lambda *s: _rng.normal(s) * 0.05)(B, S, D)), 'w_r': _w((lambda *s: _rng.normal(s) * 0.05)(D)), 'w_gate': _w((lambda *s: _rng.normal(s) * 0.05)(D, F)), 'w_up': _w((lambda *s: _rng.normal(s) * 0.05)(D, F)), 'w_down': _w((lambda *s: _rng.normal(s) * 0.05)(F, D))}
    _B_in = _B_setup()
    return {'A_x': _A_in['x'], 'A_k_cache': _A_in['k_cache'], 'A_v_cache': _A_in['v_cache'], 'A_wq': _A_in['wq'], 'A_wo': _A_in['wo'], 'B_x': _B_in['x'], 'B_w_r': _B_in['w_r'], 'B_w_gate': _B_in['w_gate'], 'B_w_up': _B_in['w_up'], 'B_w_down': _B_in['w_down'], 'c': _w((lambda *s: _rng.normal(s) * 0.05)(8, 576)), 'w_mod': _w((lambda *s: _rng.normal(s) * 0.05)(576, 6 * 576) * 576 ** (-0.5))}

def reference(A_x, A_k_cache, A_v_cache, A_wq, A_wo, B_x, B_w_r, B_w_gate, B_w_up, B_w_down, c, w_mod):

    def _A_ref(x, k_cache, v_cache, wq, wo):
        B, Sq, D = x.shape
        Hq, Dh = (32, 128)
        Hkv, Sk = (k_cache.shape[1], k_cache.shape[2])
        W = min(4096, max(256, Sk // 4))
        rep = Hq // Hkv
        q = (lambda x, *d: x.transpose(*d))((x @ wq).reshape(B, Sq, Hq, Dh), 0, 2, 1, 3)
        k = jnp.repeat(k_cache[:, :, Sk - W:, :], rep, axis=1)
        v = jnp.repeat(v_cache[:, :, Sk - W:, :], rep, axis=1)
        scores = jnp.einsum('bhqd,bhkd->bhqk', q, k) * Dh ** (-0.5)
        p = _softmax(scores, axis=-1)
        o = jnp.einsum('bhqk,bhkd->bhqd', p, v)
        return (lambda x, *d: x.transpose(*d))(o, 0, 2, 1, 3).reshape(B, Sq, Hq * Dh) @ wo

    def _B_ref(x, w_r, w_gate, w_up, w_down):
        B, S, D = x.shape
        C = 1
        r = x @ w_r
        idx = jnp.argsort(-r, axis=-1)[:, :C]
        idx_e = jnp.repeat(idx.reshape(B, C, 1), D, axis=2)
        x_sel = jnp.take_along_axis(x, idx_e, axis=1)
        g = _silu(x_sel @ w_gate)
        u = x_sel @ w_up
        y = g * u @ w_down
        r_sel = _sigmoid(jnp.take_along_axis(r, idx, axis=1))
        y = y * r_sel.reshape(B, C, 1)
        b_off = (jnp.arange(B) * S).reshape(B, 1)
        flat_idx = (idx + b_off).reshape(B * C)
        zero = (x * 0.0).reshape(B * S, D)
        upd = _scatter_add(zero, flat_idx, y.reshape(B * C, D), axis=0)
        return x + upd.reshape(B, S, D)
    x = A_x
    mod = (_silu(c) @ w_mod).reshape(c.shape[0], 6, 1, -1)
    sa, ca, ga, sb, cb, gb = (mod[:, 0].copy(), mod[:, 1].copy(), mod[:, 2].copy(), mod[:, 3].copy(), mod[:, 4].copy(), mod[:, 5].copy())
    h = _layernorm(x, axis=-1) * (1 + ca) + sa
    x = x + ga * _A_ref(h, A_k_cache, A_v_cache, A_wq, A_wo)
    h = _layernorm(x, axis=-1) * (1 + cb) + sb
    x = x + gb * _B_ref(h, B_w_r, B_w_gate, B_w_up, B_w_down)
    return x
```

```python
import functools

import jax
import jax.numpy as jnp
from jax import lax
import jax.experimental.pallas as pl
import jax.experimental.pallas.tpu as pltpu

F32 = jnp.float32
BF16 = jnp.bfloat16
_NT = (((1,), (1,)), ((), ()))


def _layernorm(x, eps=1e-5):
    m = jnp.mean(x, axis=-1, keepdims=True)
    d = x - m
    v = jnp.mean(d * d, axis=-1, keepdims=True)
    return d / jnp.sqrt(v + eps)


def _sigmoid(x):
    return 1.0 / (1.0 + jnp.exp(-x))


def make(ns=4, sr=128, wrows=8, do_compute=True, do_dma=True, nd_chunks=(128, 128, 128, 128, 64)):
    def body(x_hbm, k_hbm, v_hbm, wq_hbm, wot_hbm, wr_hbm, wg_hbm, wu_hbm, wdt_hbm, c_hbm, wmod_hbm,
             out_hbm,
             kbuf, vbuf, wq_v, wot_v, wg_v, wu_v, wdt_v, wmod_v, x_v, c_v, wr_v, q_scr, o_scr, out_v,
             kv_sem, w_sem, d_sem, s_sem):
        B, HKV, SK, DH = k_hbm.shape
        W = kbuf.shape[1]
        D = x_v.shape[1]
        n_steps = B * HKV

        def start_rows(src, dst, sem, r0, nrows, ncol):
            cw = src.shape[1] // ncol

            def one(t, carry):
                r = pl.multiple_of(r0 + t * wrows, wrows)
                for j in range(ncol):
                    pltpu.make_async_copy(
                        src.at[pl.ds(r, wrows), pl.ds(j * cw, cw)],
                        dst.at[pl.ds(r, wrows), pl.ds(j * cw, cw)], sem).start(priority=j % 2)
                return carry

            lax.fori_loop(0, nrows // wrows, one, None)

        def wait_rows(dst, sem, r0, nrows):
            d = dst.at[pl.ds(r0, nrows)]
            pltpu.make_async_copy(d, d, sem).wait()

        def start_kv(i, slot):
            h = i // B
            b = i % B
            for j in range(W // sr):
                for t, (src, dst) in enumerate(((k_hbm, kbuf), (v_hbm, vbuf))):
                    pltpu.make_async_copy(
                        src.at[b, h, pl.ds(SK - W + j * sr, sr), :],
                        dst.at[slot, pl.ds(j * sr, sr), :], kv_sem.at[t, slot]).start(priority=t)

        def wait_kv(t, slot):
            buf = (kbuf, vbuf)[t]
            pltpu.make_async_copy(buf.at[slot], buf.at[slot], kv_sem.at[t, slot]).wait()

        small = [pltpu.make_async_copy(s, d, s_sem.at[n])
                 for n, (s, d) in enumerate(((c_hbm, c_v), (x_hbm, x_v), (wr_hbm, wr_v)))]
        start_rows(wmod_hbm, wmod_v, w_sem.at[0], 0, D, 3)
        for cp in small:
            cp.start()
        start_rows(wq_hbm, wq_v, w_sem.at[1], 0, D, 2)
        if do_dma:
            lax.fori_loop(0, ns, lambda s, c: start_kv(s, s), None)
        for cp in small:
            cp.wait()
        wait_rows(wmod_v, w_sem.at[0], 0, D)

        cf = c_v[...].astype(F32)
        sc = (cf * _sigmoid(cf)).astype(BF16)
        mod = jnp.dot(sc, wmod_v[...], preferred_element_type=F32)
        sa, ca, ga, sb, cb, gb = (mod[:, n * D:(n + 1) * D] for n in range(6))
        x0 = x_v[...].astype(F32)
        h1 = (_layernorm(x0) * (1.0 + ca) + sa).astype(BF16)
        wait_rows(wq_v, w_sem.at[1], 0, D)
        q = jnp.dot(h1, wq_v[...], preferred_element_type=F32)
        for hp in range(HKV):
            q_scr[hp] = jnp.concatenate(
                [q[:, (2 * hp) * DH:(2 * hp + 1) * DH], q[:, (2 * hp + 1) * DH:(2 * hp + 2) * DH]],
                axis=0).astype(BF16)

        tail = [(wot_hbm, wot_v, w_sem.at[2], 0, D, 2),
                (wg_hbm, wg_v, w_sem.at[3], 0, D, 2),
                (wu_hbm, wu_v, w_sem.at[4], 0, D, 2)]
        r0 = 0
        dchunks = []
        for n, nr in enumerate(nd_chunks):
            dchunks.append((wdt_hbm, wdt_v, d_sem.at[n], r0, nr, 2))
            r0 += nr
        assert r0 == D
        portions = [[] for _ in range(ns)]
        portions[0].append(tail[0])
        portions[min(1, ns - 1)].append(tail[1])
        portions[min(2, ns - 1)].append(tail[2])
        portions[min(3, ns - 1)].extend(dchunks)

        scale = DH ** -0.5
        row_b = lax.broadcasted_iota(jnp.int32, (2 * B, DH), 0) % B

        def step(i, o_acc):
            slot = i % ns
            hp = i // B
            b = i % B
            if do_dma:
                wait_kv(0, slot)
            if do_compute:
                s = lax.dot_general(q_scr[hp], kbuf[slot], _NT, preferred_element_type=F32) * scale
                m = jnp.max(s, axis=-1, keepdims=True)
                p = jnp.exp(s - m)
                l = jnp.sum(p, axis=-1, keepdims=True)
            if do_dma:
                wait_kv(1, slot)
            if do_compute:
                o = jnp.dot(p.astype(BF16), vbuf[slot], preferred_element_type=F32) / l
                o_acc = jnp.where(row_b == b, o, o_acc)
                o_scr[hp] = o_acc

            if do_dma:
                @pl.when(i + ns < n_steps)
                def _():
                    start_kv(i + ns, slot)

            for n, portion in enumerate(portions):
                @pl.when(i + ns == n_steps + n)
                def _():
                    for args in portion:
                        start_rows(*args)
            return o_acc

        lax.fori_loop(0, n_steps, step, jnp.zeros((2 * B, DH), F32))

        attn = jnp.concatenate(
            [o_scr[hp, pl.ds(r * B, B), :] for hp in range(HKV) for r in range(2)], axis=1).astype(BF16)
        wait_rows(wot_v, w_sem.at[2], 0, D)
        x1 = x0 + ga * lax.dot_general(attn, wot_v[...], _NT, preferred_element_type=F32)
        h2 = _layernorm(x1) * (1.0 + cb) + sb
        h2b = h2.astype(BF16)
        wr = wr_v[...].astype(F32).reshape(1, D)
        gate = _sigmoid(jnp.sum(h2b.astype(F32) * wr, axis=-1, keepdims=True))
        wait_rows(wg_v, w_sem.at[3], 0, D)
        g = jnp.dot(h2b, wg_v[...], preferred_element_type=F32)
        g = g * _sigmoid(g)
        wait_rows(wu_v, w_sem.at[4], 0, D)
        u = jnp.dot(h2b, wu_v[...], preferred_element_type=F32)
        a = (g * u).astype(BF16)
        base = h2 + h2 * 0.0
        for (_, _, sem, r0, nr, _) in dchunks:
            wait_rows(wdt_v, sem, r0, nr)
            y = lax.dot_general(a, wdt_v[pl.ds(r0, nr), :], _NT, preferred_element_type=F32)
            sl = slice(r0, r0 + nr)
            out_v[:, sl] = (x1[:, sl] + gb[:, sl] * (base[:, sl] + y * gate)).astype(out_v.dtype)
        cp = pltpu.make_async_copy(out_v, out_hbm, s_sem.at[3])
        cp.start()
        cp.wait()

    def fn(A_x, A_k_cache, A_v_cache, A_wq, A_wo, B_x, B_w_r, B_w_gate, B_w_up, B_w_down, c, w_mod):
        del B_x
        B, _, D = A_x.shape
        _, HKV, SK, DH = A_k_cache.shape
        W = min(4096, max(256, SK // 4))
        F = B_w_gate.shape[1]
        HD = A_wq.shape[1]
        hbm = pl.BlockSpec(memory_space=pltpu.HBM)
        out = pl.pallas_call(
            body,
            out_shape=jax.ShapeDtypeStruct((B, D), A_x.dtype),
            in_specs=[hbm] * 11,
            out_specs=hbm,
            scratch_shapes=[
                pltpu.VMEM((ns, W, DH), BF16), pltpu.VMEM((ns, W, DH), BF16),
                pltpu.VMEM((D, HD), BF16), pltpu.VMEM((D, HD), BF16),
                pltpu.VMEM((D, F), BF16), pltpu.VMEM((D, F), BF16), pltpu.VMEM((D, F), BF16),
                pltpu.VMEM((D, 6 * D), BF16),
                pltpu.VMEM((B, D), BF16), pltpu.VMEM((B, D), BF16), pltpu.VMEM((D,), BF16),
                pltpu.VMEM((HKV, 2 * B, DH), BF16), pltpu.VMEM((HKV, 2 * B, DH), F32),
                pltpu.VMEM((B, D), A_x.dtype),
                pltpu.SemaphoreType.DMA((2, ns)), pltpu.SemaphoreType.DMA((5,)),
                pltpu.SemaphoreType.DMA((len(nd_chunks),)), pltpu.SemaphoreType.DMA((4,)),
            ],
            compiler_params=pltpu.CompilerParams(
                vmem_limit_bytes=100 * 1024 * 1024, disable_bounds_checks=True),
        )(A_x.reshape(B, D), A_k_cache, A_v_cache, A_wq, A_wo.T, B_w_r, B_w_gate, B_w_up, B_w_down.T, c, w_mod)
        return out.reshape(A_x.shape)

    return fn


_impl = make()


@jax.jit
def pallas_adaLN_cond__sliding_block_cached__moe_arch_mod__decode_kernel(
    A_x, A_k_cache, A_v_cache, A_wq, A_wo, B_x, B_w_r, B_w_gate, B_w_up, B_w_down, c, w_mod,
):
    return _impl(A_x, A_k_cache, A_v_cache, A_wq, A_wo, B_x, B_w_r, B_w_gate, B_w_up, B_w_down, c, w_mod)
```

```python
import contextlib

import jax
import jax.numpy as jnp
from jax import lax
import jax.experimental.pallas as pl
import jax.experimental.pallas.tpu as pltpu

F32 = jnp.float32
BF16 = jnp.bfloat16
_NT = (((1,), (1,)), ((), ()))
TR = 8


def _layernorm(x, eps=1e-5):
    m = jnp.mean(x, axis=-1, keepdims=True)
    d = x - m
    v = jnp.mean(d * d, axis=-1, keepdims=True)
    return d / jnp.sqrt(v + eps)


def _sigmoid(x):
    return 1.0 / (1.0 + jnp.exp(-x))


def make(ns=4, sr=128, pure_dma=False, scopes=False, pat='01',
         splits=(288, 288, 288, 288, 352),
         dr0=((0, 128), (128, 64), (544, 32)),
         dr1=((192, 64), (256, 128), (384, 64), (448, 64), (512, 32)),
         dorder=((0, 128), (256, 128), (128, 128), (544, 32), (384, 64), (448, 64), (512, 32)),
         look=(20, 3, 20, 20, 20), ncol=2, nosem=True):
    scope = jax.named_scope if scopes else (lambda name: contextlib.nullcontext())

    def body(x_hbm, k_hbm, v_hbm, wq_hbm, wot_hbm, wr_hbm, wg_hbm, wu_hbm, wdt_hbm, c_hbm, wmod_hbm,
             out_hbm,
             kbuf, vbuf, wq_v, wot_v, wg_v, wu_v, wdt_v, wmod_v, x_v, c_v, wr_v, q_scr, o_scr, out_v,
             kv_sem, w_sem, d_sem, s_sem):
        B, HKV, SK, DH = k_hbm.shape
        W = kbuf.shape[1]
        D = x_v.shape[1]
        n_steps = B * HKV

        def row_copies(run, t):
            src, dst, sem, r0, _ = run
            r = r0 + t * TR
            if not isinstance(r, int):
                r = pl.multiple_of(r, TR)
            tiles = src.shape[1] // 128
            cuts = [128 * -(-tiles * j // ncol) for j in range(ncol + 1)]
            out = []
            for a, b in zip(cuts[:-1], cuts[1:]):
                idx = (pl.ds(r, TR), pl.ds(a, b - a))
                out.append(pltpu.make_async_copy(src.at[idx], dst.at[idx], sem))
            return out

        class Stream:
            def __init__(self, lane0, lane1):
                self.lanes = (lane0, lane1)
                self.pos = 0
                lens = [sum(run[4] // TR for run in lane) for lane in self.lanes]
                assert lens[0] == lens[1], lens
                self.total = lens[0]

            def _locate(self, lane, k):
                for run in lane:
                    n = run[4] // TR
                    if k < n:
                        return run, k, n - k
                    k -= n

            def start(self, k0, k1, locate_at=None):
                runs = [self._locate(lane, locate_at) for lane in self.lanes]

                def one(k, carry):
                    copies = [row_copies(run, k - locate_at + t) for run, t, _ in runs]
                    for pair in zip(*copies):
                        for queue, cp in enumerate(pair):
                            cp.start(priority=queue)
                    return carry

                lax.fori_loop(k0, k1, one, None)

            def advance_to(self, pos):
                pos = min(pos, self.total)
                while self.pos < pos:
                    n = min([self._locate(lane, self.pos)[2] for lane in self.lanes] + [pos - self.pos])
                    self.start(self.pos, self.pos + n, self.pos)
                    self.pos += n

        def wait_rows(dst, sem, r0, nr):
            d = dst.at[pl.ds(r0, nr)]
            pltpu.make_async_copy(d, d, sem).wait()

        def start_kv(i, slot):
            h = i // B
            b = i % B
            n = 0
            for j in range(W // sr):
                for t, (src, dst) in enumerate(((k_hbm, kbuf), (v_hbm, vbuf))):
                    pltpu.make_async_copy(
                        src.at[b, h, pl.ds(SK - W + j * sr, sr), :],
                        dst.at[slot, pl.ds(j * sr, sr), :], kv_sem.at[t, slot]).start(
                            priority=int(pat[n % len(pat)]))
                    n += 1

        def wait_kv(t, slot):
            buf = (kbuf, vbuf)[t]
            pltpu.make_async_copy(buf.at[slot], buf.at[slot], kv_sem.at[t, slot]).wait()

        mats = [(wmod_hbm, wmod_v), (wq_hbm, wq_v), (wot_hbm, wot_v), (wg_hbm, wg_v), (wu_hbm, wu_v)]
        lo = [(s, d, w_sem.at[n], 0, splits[n]) for n, (s, d) in enumerate(mats)]
        hi = [(s, d, w_sem.at[n], splits[n], D - splits[n]) for n, (s, d) in enumerate(mats)]
        d_runs = [(wdt_hbm, wdt_v, d_sem.at[n], r0, nr) for n, (r0, nr) in enumerate(dr0 + dr1)]
        assert sum(nr for _, nr in dr0 + dr1) == D and sum(nr for _, nr in dorder) == D
        head = Stream(lo[:2], hi[:2])
        tail = Stream(lo[2:] + d_runs[:len(dr0)], hi[2:] + d_runs[len(dr0):])

        def end_of(runs):
            return sum(run[4] // TR for run in runs)

        small = [pltpu.make_async_copy(s, d, s_sem.at[n])
                 for n, (s, d) in enumerate(((c_hbm, c_v), (x_hbm, x_v), (wr_hbm, wr_v)))]
        head.advance_to(2)
        for cp in small:
            cp.start()
        head.advance_to(end_of(hi[:1]) + look[0])
        for cp in small:
            cp.wait()
        with scope('w_mod'):
            wait_rows(wmod_v, w_sem.at[0], 0, D)

        if not pure_dma:
            cf = c_v[...].astype(F32)
            sc = (cf * _sigmoid(cf)).astype(BF16)
            mod = jnp.dot(sc, wmod_v[...], preferred_element_type=F32)
            sa, ca, ga, sb, cb, gb = (mod[:, n * D:(n + 1) * D] for n in range(6))
            x0 = x_v[...].astype(F32)
            h1 = (_layernorm(x0) * (1.0 + ca) + sa).astype(BF16)
        with scope('i_q'):
            head.advance_to(head.total)
            lax.fori_loop(0, look[1], lambda s, c: start_kv(s, s), None)
        with scope('w_q'):
            wait_rows(wq_v, w_sem.at[1], 0, D)
        if not pure_dma:
            q = jnp.dot(h1, wq_v[...], preferred_element_type=F32)
            for hp in range(HKV):
                q_scr[hp] = jnp.concatenate(
                    [q[:, (2 * hp) * DH:(2 * hp + 1) * DH], q[:, (2 * hp + 1) * DH:(2 * hp + 2) * DH]],
                    axis=0).astype(BF16)
        with scope('i_kv'):
            lax.fori_loop(look[1], ns, lambda s, c: start_kv(s, s), None)

        scale = DH ** -0.5
        row_b = lax.broadcasted_iota(jnp.int32, (2 * B, DH), 0) % B
        per_step = min(8, min(lo[2][4], hi[2][4]) // TR // ns)

        def step(i, o_acc):
            slot = i % ns
            hp = i // B
            b = i % B
            wait_kv(0, slot)
            if not pure_dma:
                s = lax.dot_general(q_scr[hp], kbuf[slot], _NT, preferred_element_type=F32) * scale
                m = jnp.max(s, axis=-1, keepdims=True)
                p = jnp.exp(s - m)
                l = jnp.sum(p, axis=-1, keepdims=True)
            wait_kv(1, slot)
            if not pure_dma:
                o = jnp.dot(p.astype(BF16), vbuf[slot], preferred_element_type=F32) / l
                o_acc = jnp.where(row_b == b, o, o_acc)
                o_scr[hp] = o_acc

            @pl.when(i + ns < n_steps)
            def _():
                start_kv(i + ns, slot)

            @pl.when(i + ns >= n_steps)
            def _():
                k0 = (i + ns - n_steps) * per_step
                tail.start(k0, k0 + per_step, 0)

            return o_acc

        with scope('main'):
            lax.fori_loop(0, n_steps, step, jnp.zeros((2 * B, DH), F32))
        tail.pos = ns * per_step

        with scope('i_o'):
            tail.advance_to(end_of(hi[2:3]) + look[2])
        if not pure_dma:
            attn = jnp.concatenate(
                [o_scr[hp, pl.ds(r * B, B), :] for hp in range(HKV) for r in range(2)], axis=1).astype(BF16)
        with scope('w_o'):
            wait_rows(wot_v, w_sem.at[2], 0, D)
        if not pure_dma:
            x1 = x0 + ga * lax.dot_general(attn, wot_v[...], _NT, preferred_element_type=F32)
            h2 = _layernorm(x1) * (1.0 + cb) + sb
            h2b = h2.astype(BF16)
            wr = wr_v[...].astype(F32).reshape(1, D)
            gate = _sigmoid(jnp.sum(h2b.astype(F32) * wr, axis=-1, keepdims=True))
            base = x1 + gb * (h2 + h2 * 0.0)
            coef = gb * gate
        with scope('i_g'):
            tail.advance_to(end_of(hi[2:4]) + look[3])
        with scope('w_g'):
            wait_rows(wg_v, w_sem.at[3], 0, D)
        if not pure_dma:
            g = jnp.dot(h2b, wg_v[...], preferred_element_type=F32)
            g = g * _sigmoid(g)
        with scope('i_u'):
            tail.advance_to(end_of(hi[2:5]) + look[4])
        with scope('w_u'):
            wait_rows(wu_v, w_sem.at[4], 0, D)
        if not pure_dma:
            u = jnp.dot(h2b, wu_v[...], preferred_element_type=F32)
            a = (g * u).astype(BF16)
        with scope('i_d'):
            tail.advance_to(tail.total)
        pending = list(d_runs)
        for n, (r0, nr) in enumerate(dorder):
            with scope(f'w_d{n}'):
                for run in list(pending):
                    if run[3] < r0 + nr and r0 < run[3] + run[4]:
                        wait_rows(wdt_v, run[2], run[3], run[4])
                        pending = [x for x in pending if x is not run]
            if not pure_dma:
                y = lax.dot_general(a, wdt_v[pl.ds(r0, nr), :], _NT, preferred_element_type=F32)
                sl = slice(r0, r0 + nr)
                out_v[:, sl] = (base[:, sl] + coef[:, sl] * y).astype(out_v.dtype)
        if pure_dma:
            out_v[...] = x_v[...]
        cp = pltpu.make_async_copy(out_v, out_hbm, s_sem.at[3])
        with scope('out'):
            cp.start()
            cp.wait()

    def fn(A_x, A_k_cache, A_v_cache, A_wq, A_wo, B_x, B_w_r, B_w_gate, B_w_up, B_w_down, c, w_mod):
        del B_x
        B, _, D = A_x.shape
        _, HKV, SK, DH = A_k_cache.shape
        W = min(4096, max(256, SK // 4))
        F = B_w_gate.shape[1]
        HD = A_wq.shape[1]
        hbm = pl.BlockSpec(memory_space=pltpu.HBM)
        out = pl.pallas_call(
            body,
            out_shape=jax.ShapeDtypeStruct((B, D), A_x.dtype),
            in_specs=[hbm] * 11,
            out_specs=hbm,
            scratch_shapes=[
                pltpu.VMEM((ns, W, DH), BF16), pltpu.VMEM((ns, W, DH), BF16),
                pltpu.VMEM((D, HD), BF16), pltpu.VMEM((D, HD), BF16),
                pltpu.VMEM((D, F), BF16), pltpu.VMEM((D, F), BF16), pltpu.VMEM((D, F), BF16),
                pltpu.VMEM((D, 6 * D), BF16),
                pltpu.VMEM((B, D), BF16), pltpu.VMEM((B, D), BF16), pltpu.VMEM((D,), BF16),
                pltpu.VMEM((HKV, 2 * B, DH), BF16), pltpu.VMEM((HKV, 2 * B, DH), F32),
                pltpu.VMEM((B, D), A_x.dtype),
                pltpu.SemaphoreType.DMA((2, ns)), pltpu.SemaphoreType.DMA((5,)),
                pltpu.SemaphoreType.DMA((len(dr0) + len(dr1),)), pltpu.SemaphoreType.DMA((4,)),
            ],
            compiler_params=pltpu.CompilerParams(
                vmem_limit_bytes=100 * 1024 * 1024, disable_bounds_checks=True,
                disable_semaphore_checks=nosem),
        )(A_x.reshape(B, D), A_k_cache, A_v_cache, A_wq, A_wo.T, B_w_r, B_w_gate, B_w_up, B_w_down.T, c, w_mod)
        return out.reshape(A_x.shape)

    return fn


_impl = make(look=(28, 4, 28, 28, 28))


@jax.jit
def pallas_adaLN_cond__sliding_block_cached__moe_arch_mod__decode_kernel(
    A_x, A_k_cache, A_v_cache, A_wq, A_wo, B_x, B_w_r, B_w_gate, B_w_up, B_w_down, c, w_mod,
):
    return _impl(A_x, A_k_cache, A_v_cache, A_wq, A_wo, B_x, B_w_r, B_w_gate, B_w_up, B_w_down, c, w_mod)
```

```python
import jax
import jax.numpy as jnp
from jax import lax
import jax.experimental.pallas as pl
import jax.experimental.pallas.tpu as pltpu

F32 = jnp.float32
BF16 = jnp.bfloat16
_NT = (((1,), (1,)), ((), ()))

_TILE_ROWS = 8
_LANES = 128
_LEAD = 56
_GROUP = 8
_SPAN = 2
_SLAB = 64
_BANDS = 6
_DOWN_FETCH = (
    ((0, 3, 32, 64), (0, 3, 0, 16), (0, 3, 16, 16)),
    ((3, 3, 32, 32), (3, 3, 64, 16), (3, 3, 80, 16), (3, 1, 0, 32), (5, 1, 0, 32), (4, 1, 0, 32)),
)
_DOWN_USE = (
    (0, 3, 32, 64), (3, 3, 32, 32), (0, 3, 0, 16), (3, 3, 64, 16), (0, 3, 16, 16), (3, 3, 80, 16),
    (3, 1, 0, 32), (5, 1, 0, 32), (4, 1, 0, 32),
)
_NUM_SEMS = 4 + 6 + len(_DOWN_USE) + 4


def _layernorm(x, eps=1e-5):
    d = x - jnp.mean(x, axis=-1, keepdims=True)
    v = jnp.mean(d * d, axis=-1, keepdims=True)
    return d / jnp.sqrt(v + eps)


class _Block:
    def __init__(self, src, dst, sem, band0, bands, row0, rows, span, tiles):
        self.src, self.dst, self.sem = src, dst, sem
        self.where = (pl.ds(band0, bands), pl.ds(row0, rows))
        width, step = src.shape[2], tiles * _LANES
        self.pieces = [
            (pl.ds(band, span), pl.ds(row, _TILE_ROWS), pl.ds(col, min(step, width - col)))
            for row in range(row0, row0 + rows, _TILE_ROWS)
            for col in range(0, width, step)
            for band in range(band0, band0 + bands, span)
        ]

    def start(self, piece, queue):
        pltpu.make_async_copy(self.src.at[piece], self.dst.at[piece], self.sem).start(priority=queue)

    def wait(self):
        filled = self.dst.at[self.where]
        pltpu.make_async_copy(filled, filled, self.sem).wait()


class _Stream:
    def __init__(self, *lanes):
        self.lanes = [[(block, piece) for block in lane for piece in block.pieces] for lane in lanes]
        self.total = len(self.lanes[0])
        assert all(len(lane) == self.total for lane in self.lanes)
        self.pos = 0

    def advance_to(self, pos):
        lo, hi = self.pos, min(pos, self.total)
        if hi <= lo:
            return
        cuts = (lo, (lo + hi) // 2, hi)

        def start(part):
            for n in range(cuts[part], cuts[part + 1]):
                for queue, lane in enumerate(self.lanes):
                    block, piece = lane[n]
                    block.start(piece, queue)

        @pl.loop(0, 2)
        def _(part):
            pl.when(part == 0)(lambda: start(0))
            pl.when(part == 1)(lambda: start(1))

        self.pos = hi

    def wait(self, *blocks):
        end = max(n + 1 for lane in self.lanes for n, (b, _) in enumerate(lane) if b in blocks)
        self.advance_to(end + _LEAD)
        for block in blocks:
            block.wait()


def _block_kernel(
    x_hbm, k_hbm, v_hbm, wq_hbm, wot_hbm, wr_hbm, wg_hbm, wu_hbm, wdt_hbm, c_hbm, wmod_hbm,
    out_hbm,
    k_buf, v_buf, wq_v, wot_v, wg_v, wu_v, wdt_v, wmod_v, x_v, c_v, wr_v,
    q_scr, o_scr, act_scr, fin_scr, out_v,
    sems,
):
    batch, kv_heads, seq, head_dim = k_hbm.shape
    window = k_buf.shape[2]
    d_model = x_v.shape[1]
    band_rows = d_model // _BANDS
    spare_sems = iter(range(4, _NUM_SEMS))

    def new_sem():
        return sems.at[next(spare_sems)]

    groups_per_row = kv_heads // _GROUP
    n_groups = batch * groups_per_row
    spans = _GROUP // _SPAN
    kv_copies = window // _SLAB * spans
    copies_per_head = (kv_copies - _LEAD) // _GROUP
    assert _LEAD + _GROUP * copies_per_head == kv_copies

    def locate(group, j):
        part = group % groups_per_row
        return group // groups_per_row, (j // _SPAN * groups_per_row + part) * _SPAN + j % _SPAN

    def start_kv(group, lo, hi):
        @pl.loop(lo, hi)
        def _(n):
            row = pl.multiple_of(n // spans * _SLAB, _SLAB)
            j = n % spans * _SPAN
            b, head = locate(group, j)
            for queue, (src, dst) in enumerate(((k_hbm, k_buf), (v_hbm, v_buf))):
                pltpu.make_async_copy(
                    src.at[b, pl.ds(head, _SPAN), pl.ds(seq - window + row, _SLAB), :],
                    dst.at[group % 2, pl.ds(j, _SPAN), pl.ds(row, _SLAB), :],
                    sems.at[2 * queue + group % 2],
                ).start(priority=queue)

    def wait_kv(group):
        for queue, buf in enumerate((k_buf, v_buf)):
            filled = buf.at[group % 2]
            pltpu.make_async_copy(filled, filled, sems.at[2 * queue + group % 2]).wait()

    def side_by_side(*pairs):
        return [_Block(src, dst, new_sem(), 0, _BANDS, 0, band_rows, 2, 8) for src, dst in pairs]

    def matrix(ref):
        return ref[...].reshape(d_model, ref.shape[2])

    half = _BANDS // 2
    mod_blocks = [
        _Block(wmod_hbm, wmod_v, new_sem(), q * half, half, 0, band_rows, half, 5) for q in range(2)
    ]
    qo_blocks = side_by_side((wq_hbm, wq_v), (wot_hbm, wot_v))
    gu_blocks = side_by_side((wg_hbm, wg_v), (wu_hbm, wu_v))
    down_blocks = {
        where: _Block(wdt_hbm, wdt_v, new_sem(), *where, where[1], 18 // where[1])
        for where in _DOWN_USE
    }
    head_stream = _Stream(*zip(mod_blocks, qo_blocks))
    tail_stream = _Stream(
        *([gu_blocks[q]] + [down_blocks[where] for where in _DOWN_FETCH[q]] for q in range(2))
    )

    small = [
        pltpu.make_async_copy(src, dst, new_sem())
        for src, dst in ((c_hbm, c_v), (x_hbm, x_v), (wr_hbm, wr_v))
    ]
    head_stream.advance_to(4)
    for copy in small:
        copy.start()
    head_stream.wait(*mod_blocks)
    for copy in small:
        copy.wait()
    cond = jax.nn.silu(c_v[...].astype(F32)).astype(BF16)
    mod = jnp.dot(cond, matrix(wmod_v), preferred_element_type=F32)
    shift_a, scale_a, gate_a, shift_b, scale_b, gate_b = (
        mod[:, n * d_model:(n + 1) * d_model] for n in range(6)
    )
    x0 = x_v[...].astype(F32)
    h1 = (_layernorm(x0) * (1.0 + scale_a) + shift_a).astype(BF16)
    o_scr[...] = jnp.zeros(o_scr.shape, F32)

    head_stream.advance_to(head_stream.total)
    start_kv(0, 0, _LEAD)
    head_stream.wait(*qo_blocks)
    q = jnp.dot(h1, matrix(wq_v), preferred_element_type=F32)
    for head in range(kv_heads):
        pair = [q[:, (2 * head + r) * head_dim:(2 * head + r + 1) * head_dim] for r in range(2)]
        q_scr[head] = jnp.concatenate(pair, axis=0).astype(BF16)
    start_kv(0, _LEAD, kv_copies)

    row_batch = lax.broadcasted_iota(jnp.int32, (2 * batch, head_dim), 0) % batch

    def attend(group, j):
        b, head = locate(group, j)
        s = lax.dot_general(q_scr[head], k_buf[group % 2, j], _NT, preferred_element_type=F32)
        s = s * head_dim ** -0.5
        p = jnp.exp(s - jnp.max(s, axis=-1, keepdims=True))
        denom = jnp.sum(p, axis=-1, keepdims=True)
        o = jnp.dot(p.astype(BF16), v_buf[group % 2, j], preferred_element_type=F32) / denom
        o_scr[head] = jnp.where(row_batch == b, o, o_scr[head])

    @pl.loop(0, n_groups - 1)
    def _(group):
        start_kv(group + 1, 0, _LEAD)
        wait_kv(group)

        @pl.loop(0, _GROUP)
        def _(j):
            attend(group, j)
            lo = _LEAD + j * copies_per_head
            start_kv(group + 1, lo, lo + copies_per_head)

    tail_stream.advance_to(_LEAD)
    wait_kv(n_groups - 1)
    for j0 in range(0, _GROUP, 2):
        pl.loop(j0, j0 + 2)(lambda j: attend(n_groups - 1, j))
        tail_stream.advance_to(_LEAD + (j0 + 2) * copies_per_head)

    attn = jnp.concatenate(
        [o_scr[head, pl.ds(r * batch, batch), :] for head in range(kv_heads) for r in range(2)],
        axis=1,
    ).astype(BF16)
    x1 = x0 + gate_a * lax.dot_general(attn, matrix(wot_v), _NT, preferred_element_type=F32)
    h2 = _layernorm(x1) * (1.0 + scale_b) + shift_b
    h2_mxu = h2.astype(BF16)
    w_r = wr_v[...].astype(F32).reshape(1, d_model)
    route = jax.nn.sigmoid(jnp.sum(h2_mxu.astype(F32) * w_r, axis=-1, keepdims=True))
    fin_scr[0] = x1 + gate_b * (h2 + h2 * 0.0)
    fin_scr[1] = gate_b * route

    tail_stream.wait(*gu_blocks)
    g = jax.nn.silu(jnp.dot(h2_mxu, matrix(wg_v), preferred_element_type=F32))
    u = jnp.dot(h2_mxu, matrix(wu_v), preferred_element_type=F32)
    act_scr[...] = (g * u).astype(BF16)

    for where in _DOWN_USE:
        band0, bands, row0, rows = where
        tail_stream.wait(down_blocks[where])
        w = wdt_v[pl.ds(band0, bands), pl.ds(row0, rows), :].reshape(bands * rows, wdt_v.shape[2])
        y = lax.dot_general(act_scr[...], w, _NT, preferred_element_type=F32)
        for i in range(bands):
            cols = pl.ds((band0 + i) * band_rows + row0, rows)
            out = fin_scr[0, :, cols] + fin_scr[1, :, cols] * y[:, i * rows:(i + 1) * rows]
            out_v[:, cols] = out.astype(out_v.dtype)

    store = pltpu.make_async_copy(out_v, out_hbm, new_sem())
    store.start()
    store.wait()


@jax.jit
def pallas_adaLN_cond__sliding_block_cached__moe_arch_mod__decode_kernel(
    A_x: jax.Array,
    A_k_cache: jax.Array,
    A_v_cache: jax.Array,
    A_wq: jax.Array,
    A_wo: jax.Array,
    B_x: jax.Array,
    B_w_r: jax.Array,
    B_w_gate: jax.Array,
    B_w_up: jax.Array,
    B_w_down: jax.Array,
    c: jax.Array,
    w_mod: jax.Array,
):
    del B_x
    batch, q_len, d_model = A_x.shape
    _, kv_heads, seq, head_dim = A_k_cache.shape
    window = min(4096, max(256, seq // 4))
    assert q_len == 1 and A_wq.shape[1] == 2 * kv_heads * head_dim
    assert d_model == sum(bands * rows for _, bands, _, rows in _DOWN_USE)

    wq, wot, wg, wu, wdt, wmod = (
        w.reshape(_BANDS, d_model // _BANDS, w.shape[1])
        for w in (A_wq, A_wo.T, B_w_gate, B_w_up, B_w_down.T, w_mod)
    )
    hbm = pl.BlockSpec(memory_space=pltpu.HBM)
    out = pl.pallas_call(
        _block_kernel,
        out_shape=jax.ShapeDtypeStruct((batch, d_model), A_x.dtype),
        in_specs=[hbm] * 11,
        out_specs=hbm,
        scratch_shapes=[
            pltpu.VMEM((2, _GROUP, window, head_dim), A_k_cache.dtype),
            pltpu.VMEM((2, _GROUP, window, head_dim), A_v_cache.dtype),
            *(pltpu.VMEM(w.shape, w.dtype) for w in (wq, wot, wg, wu, wdt, wmod)),
            pltpu.VMEM((batch, d_model), A_x.dtype),
            pltpu.VMEM(c.shape, c.dtype),
            pltpu.VMEM(B_w_r.shape, B_w_r.dtype),
            pltpu.VMEM((kv_heads, 2 * batch, head_dim), BF16),
            pltpu.VMEM((kv_heads, 2 * batch, head_dim), F32),
            pltpu.VMEM((batch, B_w_gate.shape[1]), BF16),
            pltpu.VMEM((2, batch, d_model), F32),
            pltpu.VMEM((batch, d_model), A_x.dtype),
            pltpu.SemaphoreType.DMA((_NUM_SEMS,)),
        ],
        compiler_params=pltpu.CompilerParams(
            vmem_limit_bytes=80 * 1024 * 1024,
            disable_bounds_checks=True,
            disable_semaphore_checks=True,
        ),
    )(A_x.reshape(batch, d_model), A_k_cache, A_v_cache, wq, wot, B_w_r, wg, wu, wdt, c, wmod)
    return out.reshape(A_x.shape)
```

```python
import contextlib

import jax
import jax.numpy as jnp
from jax import lax
import jax.experimental.pallas as pl
import jax.experimental.pallas.tpu as pltpu

F32 = jnp.float32
BF16 = jnp.bfloat16
_NT = (((1,), (1,)), ((), ()))
TR = 8


def _layernorm(x, eps=1e-5):
    m = jnp.mean(x, axis=-1, keepdims=True)
    d = x - m
    v = jnp.mean(d * d, axis=-1, keepdims=True)
    return d / jnp.sqrt(v + eps)


def _sigmoid(x):
    return 1.0 / (1.0 + jnp.exp(-x))


def make(ns=5, nkv=(12, 12), pure_dma=False, scopes=False, pat='01',
         splits=(288, 288, 288, 288, 352),
         dr0=((0, 128), (128, 64), (544, 32)),
         dr1=((192, 64), (256, 128), (384, 64), (448, 64), (512, 32)),
         dorder=((0, 128), (256, 128), (128, 128), (544, 32), (384, 64), (448, 64), (512, 32)),
         look=(28, 4, 28, 28, 28),
         wcuts={27: (0, 14, 27), 32: (0, 16, 32), 36: (0, 18, 36)},
         lastcuts=None):
    scope = jax.named_scope if scopes else (lambda name: contextlib.nullcontext())
    n_last = len(lastcuts) - 1 if lastcuts else 0

    def body(x_hbm, k_hbm, v_hbm, wq_hbm, wot_hbm, wr_hbm, wg_hbm, wu_hbm, wdt_hbm, c_hbm, wmod_hbm,
             out_hbm,
             kbuf, vbuf, wq_v, wot_v, wg_v, wu_v, wdt_v, wmod_v, x_v, c_v, wr_v, q_scr, o_scr, a_scr, fin_v, out_v,
             kv_sem, w_sem, d_sem, s_sem):
        B, HKV, SK, DH = k_hbm.shape
        W = kbuf.shape[1]
        D = x_v.shape[1]
        n_steps = B * HKV

        def row_copies(run, t):
            src, dst, sem, r0, _ = run
            r = r0 + t * TR
            if not isinstance(r, int):
                r = pl.multiple_of(r, TR)
            cuts = [128 * t for t in wcuts[src.shape[1] // 128]]
            out = []
            for a, b in zip(cuts[:-1], cuts[1:]):
                idx = (pl.ds(r, TR), pl.ds(a, b - a))
                out.append(pltpu.make_async_copy(src.at[idx], dst.at[idx], sem))
            return out

        class Stream:
            def __init__(self, lane0, lane1):
                self.lanes = (lane0, lane1)
                self.pos = 0
                lens = [sum(run[4] // TR for run in lane) for lane in self.lanes]
                assert lens[0] == lens[1], lens
                self.total = lens[0]

            def _locate(self, lane, k):
                for run in lane:
                    n = run[4] // TR
                    if k < n:
                        return run, k, n - k
                    k -= n

            def start(self, k0, k1, locate_at=None):
                runs = [self._locate(lane, locate_at) for lane in self.lanes]

                def one(k, carry):
                    copies = [row_copies(run, k - locate_at + t) for run, t, _ in runs]
                    for pair in zip(*copies):
                        for queue, cp in enumerate(pair):
                            cp.start(priority=queue)
                    return carry

                lax.fori_loop(k0, k1, one, None)

            def advance_to(self, pos):
                pos = min(pos, self.total)
                while self.pos < pos:
                    n = min([self._locate(lane, self.pos)[2] for lane in self.lanes] + [pos - self.pos])
                    self.start(self.pos, self.pos + n, self.pos)
                    self.pos += n

        def wait_rows(dst, sem, r0, nr):
            d = dst.at[pl.ds(r0, nr)]
            pltpu.make_async_copy(d, d, sem).wait()

        def start_kv(i, slot):
            h = i // B
            b = i % B
            pieces = []
            for t, n in enumerate(nkv):
                cuts = [W // TR * j // n * TR for j in range(n + 1)] if isinstance(n, int) else n
                pieces += [(a, t, b - a) for a, b in zip(cuts[:-1], cuts[1:])]
            for r, t, nr in sorted(pieces):
                src, dst = ((k_hbm, kbuf), (v_hbm, vbuf))[t]
                pltpu.make_async_copy(
                    src.at[b, h, pl.ds(SK - W + r, nr), :],
                    dst.at[slot, pl.ds(r, nr), :], kv_sem.at[t, slot]).start(priority=int(pat[t]))

        def wait_kv(t, slot):
            buf = (kbuf, vbuf)[t]
            pltpu.make_async_copy(buf.at[slot], buf.at[slot], kv_sem.at[t, slot]).wait()

        mats = [(wmod_hbm, wmod_v), (wq_hbm, wq_v), (wot_hbm, wot_v), (wg_hbm, wg_v), (wu_hbm, wu_v)]
        lo = [(s, d, w_sem.at[n], 0, splits[n]) for n, (s, d) in enumerate(mats)]
        hi = [(s, d, w_sem.at[n], splits[n], D - splits[n]) for n, (s, d) in enumerate(mats)]
        d_runs = [(wdt_hbm, wdt_v, d_sem.at[n], r0, nr) for n, (r0, nr) in enumerate(dr0 + dr1)]
        assert sum(nr for _, nr in dr0 + dr1) == D and sum(nr for _, nr in dorder) == D
        head = Stream(lo[:2], hi[:2])
        if lastcuts:
            assert dr0[-1][1] == dr1[-1][1] and dorder[-1] == dr1[-1]
            tail = Stream(lo[2:] + d_runs[:len(dr0) - 1], hi[2:] + d_runs[len(dr0):-1])
        else:
            tail = Stream(lo[2:] + d_runs[:len(dr0)], hi[2:] + d_runs[len(dr0):])

        def end_of(runs):
            return sum(run[4] // TR for run in runs)

        small = [pltpu.make_async_copy(s, d, s_sem.at[n])
                 for n, (s, d) in enumerate(((c_hbm, c_v), (x_hbm, x_v), (wr_hbm, wr_v)))]
        head.advance_to(2)
        for cp in small:
            cp.start()
        head.advance_to(end_of(hi[:1]) + look[0])
        for cp in small:
            cp.wait()
        with scope('w_mod'):
            wait_rows(wmod_v, w_sem.at[0], 0, D)

        if not pure_dma:
            cf = c_v[...].astype(F32)
            sc = (cf * _sigmoid(cf)).astype(BF16)
            mod = jnp.dot(sc, wmod_v[...], preferred_element_type=F32)
            sa, ca, ga, sb, cb, gb = (mod[:, n * D:(n + 1) * D] for n in range(6))
            x0 = x_v[...].astype(F32)
            h1 = (_layernorm(x0) * (1.0 + ca) + sa).astype(BF16)
        with scope('i_q'):
            head.advance_to(head.total)
            lax.fori_loop(0, look[1], lambda s, c: start_kv(s, s), None)
        with scope('w_q'):
            wait_rows(wq_v, w_sem.at[1], 0, D)
        if not pure_dma:
            q = jnp.dot(h1, wq_v[...], preferred_element_type=F32)
            for hp in range(HKV):
                q_scr[hp] = jnp.concatenate(
                    [q[:, (2 * hp) * DH:(2 * hp + 1) * DH], q[:, (2 * hp + 1) * DH:(2 * hp + 2) * DH]],
                    axis=0).astype(BF16)
        with scope('i_kv'):
            lax.fori_loop(look[1], ns, lambda s, c: start_kv(s, s), None)

        scale = DH ** -0.5
        row_b = lax.broadcasted_iota(jnp.int32, (2 * B, DH), 0) % B
        per_step = min(nkv[0] // 2 if isinstance(nkv[0], int) else 6,
                       min(lo[2][4], hi[2][4]) // TR // ns)

        def step(i, o_acc):
            slot = i % ns
            hp = i // B
            b = i % B
            wait_kv(0, slot)
            if not pure_dma:
                s = lax.dot_general(q_scr[hp], kbuf[slot], _NT, preferred_element_type=F32) * scale
                m = jnp.max(s, axis=-1, keepdims=True)
                p = jnp.exp(s - m)
                l = jnp.sum(p, axis=-1, keepdims=True)
            wait_kv(1, slot)
            if not pure_dma:
                o = jnp.dot(p.astype(BF16), vbuf[slot], preferred_element_type=F32) / l
                o_acc = jnp.where(row_b == b, o, o_acc)
                o_scr[hp] = o_acc

            @pl.when(i + ns < n_steps)
            def _():
                start_kv(i + ns, slot)

            @pl.when(i + ns >= n_steps)
            def _():
                k0 = (i + ns - n_steps) * per_step
                tail.start(k0, k0 + per_step, 0)

            return o_acc

        with scope('main'):
            lax.fori_loop(0, n_steps, step, jnp.zeros((2 * B, DH), F32))
        tail.pos = ns * per_step

        with scope('i_o'):
            tail.advance_to(end_of(hi[2:3]) + look[2])
        if not pure_dma:
            attn = jnp.concatenate(
                [o_scr[hp, pl.ds(r * B, B), :] for hp in range(HKV) for r in range(2)], axis=1).astype(BF16)
        with scope('w_o'):
            wait_rows(wot_v, w_sem.at[2], 0, D)
        if not pure_dma:
            x1 = x0 + ga * lax.dot_general(attn, wot_v[...], _NT, preferred_element_type=F32)
            h2 = _layernorm(x1) * (1.0 + cb) + sb
            h2b = h2.astype(BF16)
            wr = wr_v[...].astype(F32).reshape(1, D)
            gate = _sigmoid(jnp.sum(h2b.astype(F32) * wr, axis=-1, keepdims=True))
            fin_v[0] = x1 + gb * (h2 + h2 * 0.0)
            fin_v[1] = gb * gate
        with scope('i_g'):
            tail.advance_to(end_of(hi[2:4]) + look[3])
        with scope('w_g'):
            wait_rows(wg_v, w_sem.at[3], 0, D)
        if not pure_dma:
            g = jnp.dot(h2b, wg_v[...], preferred_element_type=F32)
            g = g * _sigmoid(g)
        with scope('i_u'):
            tail.advance_to(end_of(hi[2:5]) + look[4])
        with scope('w_u'):
            wait_rows(wu_v, w_sem.at[4], 0, D)
        if not pure_dma:
            u = jnp.dot(h2b, wu_v[...], preferred_element_type=F32)
            a_scr[...] = (g * u).astype(BF16)
        with scope('i_d'):
            tail.advance_to(tail.total)
            if lastcuts:
                nd = len(d_runs)
                for j, (c0, c1) in enumerate(zip(lastcuts[:-1], lastcuts[1:])):
                    for t in range(dr1[-1][1] // TR):
                        for queue, (r0, sem) in enumerate(((dr0[-1][0], d_sem.at[len(dr0) - 1]),
                                                           (dr1[-1][0], d_sem.at[nd - 1 + j]))):
                            idx = (pl.ds(r0 + t * TR, TR), pl.ds(128 * c0, 128 * (c1 - c0)))
                            pltpu.make_async_copy(wdt_hbm.at[idx], wdt_v.at[idx], sem).start(priority=queue)
        pending = list(d_runs)
        for n, (r0, nr) in enumerate(dorder):
            sl = slice(r0, r0 + nr)
            if lastcuts and n == len(dorder) - 1:
                y = None
                for j, (c0, c1) in enumerate(zip(lastcuts[:-1], lastcuts[1:])):
                    cs = pl.ds(128 * c0, 128 * (c1 - c0))
                    d = wdt_v.at[pl.ds(r0, nr), cs]
                    with scope(f'w_l{j}'):
                        pltpu.make_async_copy(d, d, d_sem.at[len(d_runs) - 1 + j]).wait()
                    if not pure_dma:
                        part = lax.dot_general(a_scr[:, cs], d[...], _NT, preferred_element_type=F32)
                        y = part if y is None else y + part
            else:
                with scope(f'w_d{n}'):
                    for run in list(pending):
                        if run[3] < r0 + nr and r0 < run[3] + run[4]:
                            wait_rows(wdt_v, run[2], run[3], run[4])
                            pending = [x for x in pending if x is not run]
                if not pure_dma:
                    y = lax.dot_general(a_scr[...], wdt_v[pl.ds(r0, nr), :], _NT, preferred_element_type=F32)
            if not pure_dma:
                out_v[:, sl] = (fin_v[0, :, sl] + fin_v[1, :, sl] * y).astype(out_v.dtype)
        if pure_dma:
            out_v[...] = x_v[...]
        cp = pltpu.make_async_copy(out_v, out_hbm, s_sem.at[3])
        with scope('out'):
            cp.start()
            cp.wait()

    def fn(A_x, A_k_cache, A_v_cache, A_wq, A_wo, B_x, B_w_r, B_w_gate, B_w_up, B_w_down, c, w_mod):
        del B_x
        B, _, D = A_x.shape
        _, HKV, SK, DH = A_k_cache.shape
        W = min(4096, max(256, SK // 4))
        F = B_w_gate.shape[1]
        HD = A_wq.shape[1]
        hbm = pl.BlockSpec(memory_space=pltpu.HBM)
        out = pl.pallas_call(
            body,
            out_shape=jax.ShapeDtypeStruct((B, D), A_x.dtype),
            in_specs=[hbm] * 11,
            out_specs=hbm,
            scratch_shapes=[
                pltpu.VMEM((ns, W, DH), BF16), pltpu.VMEM((ns, W, DH), BF16),
                pltpu.VMEM((D, HD), BF16), pltpu.VMEM((D, HD), BF16),
                pltpu.VMEM((D, F), BF16), pltpu.VMEM((D, F), BF16), pltpu.VMEM((D, F), BF16),
                pltpu.VMEM((D, 6 * D), BF16),
                pltpu.VMEM((B, D), BF16), pltpu.VMEM((B, D), BF16), pltpu.VMEM((D,), BF16),
                pltpu.VMEM((HKV, 2 * B, DH), BF16), pltpu.VMEM((HKV, 2 * B, DH), F32),
                pltpu.VMEM((B, F), BF16), pltpu.VMEM((2, B, D), F32),
                pltpu.VMEM((B, D), A_x.dtype),
                pltpu.SemaphoreType.DMA((2, ns)), pltpu.SemaphoreType.DMA((5,)),
                pltpu.SemaphoreType.DMA((len(dr0) + len(dr1) + n_last,)), pltpu.SemaphoreType.DMA((4,)),
            ],
            compiler_params=pltpu.CompilerParams(
                vmem_limit_bytes=100 * 1024 * 1024, disable_bounds_checks=True,
                disable_semaphore_checks=True),
        )(A_x.reshape(B, D), A_k_cache, A_v_cache, A_wq, A_wo.T, B_w_r, B_w_gate, B_w_up, B_w_down.T, c, w_mod)
        return out.reshape(A_x.shape)

    return fn


_impl = make(nkv=((0, 144, 288, 432, 576, 720, 864, 1008, 1152, 1296, 1440, 1584, 1728, 1888, 2048), (0, 168, 336, 512, 680, 848, 1024, 1192, 1360, 1536, 1704, 1872, 2048)))


@jax.jit
def pallas_adaLN_cond__sliding_block_cached__moe_arch_mod__decode_kernel(
    A_x, A_k_cache, A_v_cache, A_wq, A_wo, B_x, B_w_r, B_w_gate, B_w_up, B_w_down, c, w_mod,
):
    return _impl(A_x, A_k_cache, A_v_cache, A_wq, A_wo, B_x, B_w_r, B_w_gate, B_w_up, B_w_down, c, w_mod)
```

```python
import jax
import jax.numpy as jnp
from jax import lax
import jax.experimental.pallas as pl
import jax.experimental.pallas.tpu as pltpu

F32 = jnp.float32
BF16 = jnp.bfloat16
_NT = (((1,), (1,)), ((), ()))

_TILE_ROWS = 8
_SLOTS = 5
_K_CUTS = (0, 144, 288, 432, 576, 720, 864, 1008, 1152, 1296, 1440, 1584, 1728, 1888, 2048)
_V_CUTS = (0, 168, 336, 512, 680, 848, 1024, 1192, 1360, 1536, 1704, 1872, 2048)
_LOOKAHEAD = 28
_SPLITS = (288, 288, 288, 288, 352)
_DOWN_RUNS = (
    ((0, 128), (128, 64), (544, 32)),
    ((192, 64), (256, 128), (384, 64), (448, 64), (512, 32)),
)
_DOWN_ORDER = ((0, 128), (256, 128), (128, 128), (544, 32), (384, 64), (448, 64), (512, 32))


def _layernorm(x, eps=1e-5):
    d = x - jnp.mean(x, axis=-1, keepdims=True)
    v = jnp.mean(d * d, axis=-1, keepdims=True)
    return d / jnp.sqrt(v + eps)


class _Run:
    def __init__(self, src, dst, sem, row0, rows):
        self.src, self.dst, self.sem, self.row0, self.rows = src, dst, sem, row0, rows
        self.strips = rows // _TILE_ROWS

    def strip_copies(self, strip):
        rows = pl.ds(pl.multiple_of(self.row0 + strip * _TILE_ROWS, _TILE_ROWS), _TILE_ROWS)
        width = self.src.shape[1]
        half = (width // 128 + 1) // 2 * 128
        return [
            pltpu.make_async_copy(self.src.at[rows, cols], self.dst.at[rows, cols], self.sem)
            for cols in (pl.ds(0, half), pl.ds(half, width - half))
        ]

    def wait(self):
        filled = self.dst.at[pl.ds(self.row0, self.rows)]
        pltpu.make_async_copy(filled, filled, self.sem).wait()


class _Stream:
    def __init__(self, *lanes):
        self.lanes = lanes
        self.pos = 0
        totals = [sum(run.strips for run in lane) for lane in lanes]
        assert totals[0] == totals[1], totals
        self.total = totals[0]

    def end_of(self, *runs):
        end = 0
        for lane in self.lanes:
            pos = 0
            for run in lane:
                pos += run.strips
                if run in runs:
                    end = max(end, pos)
        return end

    def _runs_at(self, pos):
        found = []
        for lane in self.lanes:
            first = 0
            for run in lane:
                if pos < first + run.strips:
                    found.append((run, first))
                    break
                first += run.strips
        return found

    def start(self, lo, hi):
        runs = self._runs_at(self.pos)

        @pl.loop(lo, hi)
        def _(pos):
            for pair in zip(*(run.strip_copies(pos - first) for run, first in runs)):
                for queue, copy in enumerate(pair):
                    copy.start(priority=queue)

    def advance_to(self, pos):
        pos = min(pos, self.total)
        while self.pos < pos:
            stop = min([pos] + [first + run.strips for run, first in self._runs_at(self.pos)])
            self.start(self.pos, stop)
            self.pos = stop


def _block_kernel(
    x_hbm, k_hbm, v_hbm, wq_hbm, wot_hbm, wr_hbm, wg_hbm, wu_hbm, wdt_hbm, c_hbm, wmod_hbm,
    out_hbm,
    k_buf, v_buf, wq_v, wot_v, wg_v, wu_v, wdt_v, wmod_v, x_v, c_v, wr_v,
    q_scr, o_scr, act_scr, fin_scr, out_v,
    kv_sem, w_sem, down_sem, small_sem,
):
    batch, kv_heads, seq, head_dim = k_hbm.shape
    window = k_buf.shape[1]
    d_model = x_v.shape[1]
    n_steps = batch * kv_heads

    def start_kv(step, slot):
        head, b = step // batch, step % batch
        pieces = sorted(
            (lo, queue, hi - lo)
            for queue, cuts in enumerate((_K_CUTS, _V_CUTS))
            for lo, hi in zip(cuts[:-1], cuts[1:])
        )
        for lo, queue, rows in pieces:
            src, dst = ((k_hbm, k_buf), (v_hbm, v_buf))[queue]
            pltpu.make_async_copy(
                src.at[b, head, pl.ds(seq - window + lo, rows), :],
                dst.at[slot, pl.ds(lo, rows), :],
                kv_sem.at[queue, slot],
            ).start(priority=queue)

    def wait_kv(which, slot):
        buf = (k_buf, v_buf)[which].at[slot]
        pltpu.make_async_copy(buf, buf, kv_sem.at[which, slot]).wait()

    def wait_weight(n):
        pltpu.make_async_copy(weights[n][1], weights[n][1], w_sem.at[n]).wait()

    weights = ((wmod_hbm, wmod_v), (wq_hbm, wq_v), (wot_hbm, wot_v), (wg_hbm, wg_v), (wu_hbm, wu_v))
    top = [_Run(s, d, w_sem.at[n], 0, _SPLITS[n]) for n, (s, d) in enumerate(weights)]
    bottom = [
        _Run(s, d, w_sem.at[n], _SPLITS[n], d_model - _SPLITS[n]) for n, (s, d) in enumerate(weights)
    ]
    down = [
        _Run(wdt_hbm, wdt_v, down_sem.at[n], row0, rows)
        for n, (row0, rows) in enumerate(_DOWN_RUNS[0] + _DOWN_RUNS[1])
    ]
    head_stream = _Stream(top[:2], bottom[:2])
    tail_stream = _Stream(
        top[2:] + down[: len(_DOWN_RUNS[0])], bottom[2:] + down[len(_DOWN_RUNS[0]):]
    )

    def queue_past(stream, n):
        stream.advance_to(
            max(stream.end_of(top[n], bottom[n]), stream.end_of(bottom[n]) + _LOOKAHEAD)
        )

    small = [
        pltpu.make_async_copy(src, dst, small_sem.at[n])
        for n, (src, dst) in enumerate(((c_hbm, c_v), (x_hbm, x_v), (wr_hbm, wr_v)))
    ]
    head_stream.advance_to(2)
    for copy in small:
        copy.start()
    queue_past(head_stream, 0)
    for copy in small:
        copy.wait()
    wait_weight(0)
    cond = jax.nn.silu(c_v[...].astype(F32)).astype(BF16)
    mod = jnp.dot(cond, wmod_v[...], preferred_element_type=F32)
    shift_a, scale_a, gate_a, shift_b, scale_b, gate_b = (
        mod[:, n * d_model:(n + 1) * d_model] for n in range(6)
    )
    x0 = x_v[...].astype(F32)
    h1 = (_layernorm(x0) * (1.0 + scale_a) + shift_a).astype(BF16)

    head_stream.advance_to(head_stream.total)
    pl.loop(0, _SLOTS - 1)(lambda s: start_kv(s, s))
    wait_weight(1)
    q = jnp.dot(h1, wq_v[...], preferred_element_type=F32)
    for head in range(kv_heads):
        pair = [q[:, (2 * head + r) * head_dim:(2 * head + r + 1) * head_dim] for r in range(2)]
        q_scr[head] = jnp.concatenate(pair, axis=0).astype(BF16)
    start_kv(_SLOTS - 1, _SLOTS - 1)

    row_batch = lax.broadcasted_iota(jnp.int32, (2 * batch, head_dim), 0) % batch
    strips_per_step = min(top[2].strips, bottom[2].strips) // _SLOTS

    def attend(step, o_rows):
        slot = step % _SLOTS
        head, b = step // batch, step % batch
        wait_kv(0, slot)
        s = lax.dot_general(q_scr[head], k_buf[slot], _NT, preferred_element_type=F32)
        s = s * head_dim ** -0.5
        p = jnp.exp(s - jnp.max(s, axis=-1, keepdims=True))
        denom = jnp.sum(p, axis=-1, keepdims=True)
        wait_kv(1, slot)
        o = jnp.dot(p.astype(BF16), v_buf[slot], preferred_element_type=F32) / denom
        o_rows = jnp.where(row_batch == b, o, o_rows)
        o_scr[head] = o_rows

        @pl.when(step + _SLOTS < n_steps)
        def _():
            start_kv(step + _SLOTS, slot)

        @pl.when(step + _SLOTS >= n_steps)
        def _():
            lo = (step + _SLOTS - n_steps) * strips_per_step
            tail_stream.start(lo, lo + strips_per_step)

        return o_rows

    lax.fori_loop(0, n_steps, attend, jnp.zeros((2 * batch, head_dim), F32))
    tail_stream.pos = _SLOTS * strips_per_step

    queue_past(tail_stream, 2)
    attn = jnp.concatenate(
        [o_scr[head, pl.ds(r * batch, batch), :] for head in range(kv_heads) for r in range(2)],
        axis=1,
    ).astype(BF16)
    wait_weight(2)
    x1 = x0 + gate_a * lax.dot_general(attn, wot_v[...], _NT, preferred_element_type=F32)
    h2 = _layernorm(x1) * (1.0 + scale_b) + shift_b
    h2_mxu = h2.astype(BF16)
    w_r = wr_v[...].astype(F32).reshape(1, d_model)
    route = jax.nn.sigmoid(jnp.sum(h2_mxu.astype(F32) * w_r, axis=-1, keepdims=True))
    fin_scr[0] = x1 + gate_b * (h2 + h2 * 0.0)
    fin_scr[1] = gate_b * route

    queue_past(tail_stream, 3)
    wait_weight(3)
    g = jax.nn.silu(jnp.dot(h2_mxu, wg_v[...], preferred_element_type=F32))
    queue_past(tail_stream, 4)
    wait_weight(4)
    u = jnp.dot(h2_mxu, wu_v[...], preferred_element_type=F32)
    act_scr[...] = (g * u).astype(BF16)

    tail_stream.advance_to(tail_stream.total)
    for row0, rows in _DOWN_ORDER:
        for run in [r for r in down if r.row0 < row0 + rows and row0 < r.row0 + r.rows]:
            run.wait()
            down.remove(run)
        y = lax.dot_general(
            act_scr[...], wdt_v[pl.ds(row0, rows), :], _NT, preferred_element_type=F32
        )
        cols = slice(row0, row0 + rows)
        out_v[:, cols] = (fin_scr[0, :, cols] + fin_scr[1, :, cols] * y).astype(out_v.dtype)

    store = pltpu.make_async_copy(out_v, out_hbm, small_sem.at[3])
    store.start()
    store.wait()


@jax.jit
def pallas_adaLN_cond__sliding_block_cached__moe_arch_mod__decode_kernel(
    A_x: jax.Array,
    A_k_cache: jax.Array,
    A_v_cache: jax.Array,
    A_wq: jax.Array,
    A_wo: jax.Array,
    B_x: jax.Array,
    B_w_r: jax.Array,
    B_w_gate: jax.Array,
    B_w_up: jax.Array,
    B_w_down: jax.Array,
    c: jax.Array,
    w_mod: jax.Array,
):
    del B_x
    batch, q_len, d_model = A_x.shape
    _, kv_heads, seq, head_dim = A_k_cache.shape
    window = min(4096, max(256, seq // 4))
    d_attn = A_wq.shape[1]
    d_ffn = B_w_gate.shape[1]
    assert q_len == 1 and d_attn == 2 * kv_heads * head_dim
    assert window == _K_CUTS[-1] == _V_CUTS[-1]
    assert d_model == sum(rows for _, rows in _DOWN_ORDER)
    assert d_model == sum(rows for _, rows in _DOWN_RUNS[0] + _DOWN_RUNS[1])

    hbm = pl.BlockSpec(memory_space=pltpu.HBM)
    out = pl.pallas_call(
        _block_kernel,
        out_shape=jax.ShapeDtypeStruct((batch, d_model), A_x.dtype),
        in_specs=[hbm] * 11,
        out_specs=hbm,
        scratch_shapes=[
            pltpu.VMEM((_SLOTS, window, head_dim), A_k_cache.dtype),
            pltpu.VMEM((_SLOTS, window, head_dim), A_v_cache.dtype),
            pltpu.VMEM((d_model, d_attn), A_wq.dtype),
            pltpu.VMEM((d_model, d_attn), A_wo.dtype),
            pltpu.VMEM((d_model, d_ffn), B_w_gate.dtype),
            pltpu.VMEM((d_model, d_ffn), B_w_up.dtype),
            pltpu.VMEM((d_model, d_ffn), B_w_down.dtype),
            pltpu.VMEM(w_mod.shape, w_mod.dtype),
            pltpu.VMEM((batch, d_model), A_x.dtype),
            pltpu.VMEM(c.shape, c.dtype),
            pltpu.VMEM(B_w_r.shape, B_w_r.dtype),
            pltpu.VMEM((kv_heads, 2 * batch, head_dim), BF16),
            pltpu.VMEM((kv_heads, 2 * batch, head_dim), F32),
            pltpu.VMEM((batch, d_ffn), BF16),
            pltpu.VMEM((2, batch, d_model), F32),
            pltpu.VMEM((batch, d_model), A_x.dtype),
            pltpu.SemaphoreType.DMA((2, _SLOTS)),
            pltpu.SemaphoreType.DMA((len(_SPLITS),)),
            pltpu.SemaphoreType.DMA((len(_DOWN_RUNS[0]) + len(_DOWN_RUNS[1]),)),
            pltpu.SemaphoreType.DMA((4,)),
        ],
        compiler_params=pltpu.CompilerParams(
            vmem_limit_bytes=64 * 1024 * 1024,
            disable_bounds_checks=True,
            disable_semaphore_checks=True,
        ),
    )(
        A_x.reshape(batch, d_model), A_k_cache, A_v_cache, A_wq, A_wo.T,
        B_w_r, B_w_gate, B_w_up, B_w_down.T, c, w_mod,
    )
    return out.reshape(A_x.shape)
```

```python
import jax
import jax.numpy as jnp
from jax import lax
import jax.experimental.pallas as pl
import jax.experimental.pallas.tpu as pltpu

F32 = jnp.float32
BF16 = jnp.bfloat16
_NT = (((1,), (1,)), ((), ()))

_TILE_ROWS = 8
_LANES = 128
_GROUP = 8
_SLAB = 16
_LEAD = 56
_BANDS = 6
_TILES = {'mod': (5,), 'q': (6,), 'o': (6,), 'gu': (2, 3), 'd': (6,)}
_ORDER = 'bh'
_PURE = False
_SCOPES = False
_DOWN_RUNS = (
    ((0, 3, 32, 32, (6,)), (0, 3, 64, 32, (6,)), (0, 3, 0, 32, (6,))),
    ((3, 3, 32, 32, (6,)), (3, 3, 64, 32, (6,)), (3, 1, 0, 32, (18,)), (5, 1, 0, 32, (18,)), (4, 1, 0, 32, (18,))),
)
_DOWN_ORDER = ((0, 6, 32, 32), (0, 6, 64, 32), (0, 3, 0, 32), (3, 1, 0, 32), (5, 1, 0, 32), (4, 1, 0, 32))


def _scope(name):
    import contextlib
    return jax.named_scope(name) if _SCOPES else contextlib.nullcontext()


def _layernorm(x, eps=1e-5):
    d = x - jnp.mean(x, axis=-1, keepdims=True)
    v = jnp.mean(d * d, axis=-1, keepdims=True)
    return d / jnp.sqrt(v + eps)


class _Run:
    def __init__(self, src, dst, sem, band0, bands, row0, rows, tiles):
        self.src, self.dst, self.sem = src, dst, sem
        self.band0, self.bands, self.row0, self.rows = band0, bands, row0, rows
        cols, col = [], 0
        while col < src.shape[2]:
            width = min(tiles[len(cols) % len(tiles)] * _LANES, src.shape[2] - col)
            cols.append(pl.ds(col, width))
            col += width
        self.pieces = [
            (self, (pl.ds(band0, bands), pl.ds(row, _TILE_ROWS), c))
            for row in range(row0, row0 + rows, _TILE_ROWS) for c in cols
        ]

    def overlaps(self, band0, bands, row0, rows):
        return (self.band0 < band0 + bands and band0 < self.band0 + self.bands
                and self.row0 < row0 + rows and row0 < self.row0 + self.rows)

    def wait(self):
        filled = self.dst.at[pl.ds(self.band0, self.bands), pl.ds(self.row0, self.rows)]
        pltpu.make_async_copy(filled, filled, self.sem).wait()


class _Stream:
    def __init__(self, *lanes):
        self.lanes = [[piece for run in lane for piece in run.pieces] for lane in lanes]
        self.total = max(len(lane) for lane in self.lanes)
        self.pos = 0

    def advance_to(self, pos):
        pos = min(pos, self.total)
        for n in range(self.pos, pos):
            for queue, lane in enumerate(self.lanes):
                if n < len(lane):
                    run, idx = lane[n]
                    pltpu.make_async_copy(run.src.at[idx], run.dst.at[idx], run.sem).start(priority=queue)
        self.pos = max(self.pos, pos)

    def wait(self, *runs):
        end = max(n + 1 for lane in self.lanes for n, (run, _) in enumerate(lane) if run in runs)
        with _scope('issue'):
            self.advance_to(end + _LEAD)
        for run in runs:
            with _scope('wait'):
                run.wait()


def _block_kernel(
    x_hbm, k_hbm, v_hbm, wq_hbm, wot_hbm, wr_hbm, wg_hbm, wu_hbm, wdt_hbm, c_hbm, wmod_hbm,
    out_hbm,
    k_buf, v_buf, wq_v, wot_v, wg_v, wu_v, wdt_v, wmod_v, x_v, c_v, wr_v,
    q_scr, o_scr, act_scr, fin_scr, out_v,
    sems,
):
    spare = iter(range(4, sems.shape[0]))

    def new_sem():
        return sems.at[next(spare)]

    batch, kv_heads, seq, head_dim = k_hbm.shape
    window = k_buf.shape[2]
    d_model = x_v.shape[1]
    band_rows = d_model // _BANDS
    per_batch = kv_heads // _GROUP
    n_groups = batch * per_batch
    slabs = window // _SLAB
    slabs_per_head = (slabs - _LEAD) // _GROUP
    assert _LEAD + _GROUP * slabs_per_head == slabs

    def locate(group):
        if _ORDER == 'bh':
            return group // per_batch, group % per_batch * _GROUP
        return group % batch, group // batch * _GROUP

    def start_kv(group, lo, hi):
        b, head0 = locate(group)

        @pl.loop(lo, hi)
        def _(slab):
            row = pl.multiple_of(slab * _SLAB, _SLAB)
            for queue, (src, dst) in enumerate(((k_hbm, k_buf), (v_hbm, v_buf))):
                pltpu.make_async_copy(
                    src.at[b, pl.ds(head0, _GROUP), pl.ds(seq - window + row, _SLAB), :],
                    dst.at[group % 2, :, pl.ds(row, _SLAB), :],
                    sems.at[2 * queue + group % 2],
                ).start(priority=queue)

    def wait_kv(group):
        for queue, buf in enumerate((k_buf, v_buf)):
            filled = buf.at[group % 2]
            pltpu.make_async_copy(filled, filled, sems.at[2 * queue + group % 2]).wait()

    def halves(src, dst, n, tiles):
        half = _BANDS // 2
        return [_Run(src, dst, new_sem(), q * half, half, 0, band_rows, tiles) for q in range(2)]

    def matrix(ref):
        return ref[...].reshape(d_model, ref.shape[2])

    mod_runs = halves(wmod_hbm, wmod_v, 0, _TILES['mod'])
    q_runs = halves(wq_hbm, wq_v, 1, _TILES['q'])
    o_runs = halves(wot_hbm, wot_v, 2, _TILES['o'])
    gu_runs = [
        _Run(src, dst, new_sem(), 0, _BANDS, 0, band_rows, _TILES['gu'])
        for q, (src, dst) in enumerate(((wg_hbm, wg_v), (wu_hbm, wu_v)))
    ]
    down_runs = [
        [_Run(wdt_hbm, wdt_v, new_sem(), *spec) for n, spec in enumerate(lane)]
        for q, lane in enumerate(_DOWN_RUNS)
    ]
    head_stream = _Stream(*zip(mod_runs, q_runs))
    tail_stream = _Stream(*([o_runs[q], gu_runs[q]] + down_runs[q] for q in range(2)))

    small = [
        pltpu.make_async_copy(src, dst, new_sem())
        for n, (src, dst) in enumerate(((c_hbm, c_v), (x_hbm, x_v), (wr_hbm, wr_v)))
    ]
    head_stream.advance_to(4)
    for copy in small:
        copy.start()
    with _scope('w_mod'):
        head_stream.wait(*mod_runs)
    for copy in small:
        copy.wait()
    cond = jax.nn.silu(c_v[...].astype(F32)).astype(BF16)
    mod = jnp.dot(cond, matrix(wmod_v), preferred_element_type=F32)
    shift_a, scale_a, gate_a, shift_b, scale_b, gate_b = (
        mod[:, n * d_model:(n + 1) * d_model] for n in range(6)
    )
    x0 = x_v[...].astype(F32)
    h1 = (_layernorm(x0) * (1.0 + scale_a) + shift_a).astype(BF16)
    o_scr[...] = jnp.zeros(o_scr.shape, F32)

    with _scope('w_q'):
        head_stream.advance_to(head_stream.total)
        start_kv(0, 0, _LEAD)
        head_stream.wait(*q_runs)
    q = jnp.dot(h1, matrix(wq_v), preferred_element_type=F32)
    for head in range(kv_heads):
        pair = [q[:, (2 * head + r) * head_dim:(2 * head + r + 1) * head_dim] for r in range(2)]
        q_scr[head] = jnp.concatenate(pair, axis=0).astype(BF16)
    with _scope('i_kv0'):
        start_kv(0, _LEAD, slabs)

    row_batch = lax.broadcasted_iota(jnp.int32, (2 * batch, head_dim), 0) % batch

    def attend(group, j):
        if _PURE:
            return
        b, head0 = locate(group)
        head = head0 + j
        s = lax.dot_general(q_scr[head], k_buf[group % 2, j], _NT, preferred_element_type=F32)
        s = s * head_dim ** -0.5
        p = jnp.exp(s - jnp.max(s, axis=-1, keepdims=True))
        denom = jnp.sum(p, axis=-1, keepdims=True)
        o = jnp.dot(p.astype(BF16), v_buf[group % 2, j], preferred_element_type=F32) / denom
        o_scr[head] = jnp.where(row_batch == b, o, o_scr[head])

    with _scope('main'):
        @pl.loop(0, n_groups - 1)
        def _(group):
            start_kv(group + 1, 0, _LEAD)
            wait_kv(group)

            @pl.loop(0, _GROUP)
            def _(j):
                attend(group, j)
                lo = _LEAD + j * slabs_per_head
                start_kv(group + 1, lo, lo + slabs_per_head)

    with _scope('last'):
        tail_stream.advance_to(_LEAD)
        wait_kv(n_groups - 1)
        for j in range(0, _GROUP, 2):
            pl.loop(j, j + 2)(lambda jj: attend(n_groups - 1, jj))
            tail_stream.advance_to(_LEAD + (j + 2) * slabs_per_head)

    with _scope('w_o'):
        tail_stream.wait(*o_runs)
    attn = jnp.concatenate(
        [o_scr[head, pl.ds(r * batch, batch), :] for head in range(kv_heads) for r in range(2)],
        axis=1,
    ).astype(BF16)
    x1 = x0 + gate_a * lax.dot_general(attn, matrix(wot_v), _NT, preferred_element_type=F32)
    h2 = _layernorm(x1) * (1.0 + scale_b) + shift_b
    h2_mxu = h2.astype(BF16)
    w_r = wr_v[...].astype(F32).reshape(1, d_model)
    route = jax.nn.sigmoid(jnp.sum(h2_mxu.astype(F32) * w_r, axis=-1, keepdims=True))
    fin_scr[0] = x1 + gate_b * (h2 + h2 * 0.0)
    fin_scr[1] = gate_b * route

    with _scope('w_gu'):
        tail_stream.wait(*gu_runs)
    g = jax.nn.silu(jnp.dot(h2_mxu, matrix(wg_v), preferred_element_type=F32))
    u = jnp.dot(h2_mxu, matrix(wu_v), preferred_element_type=F32)
    act_scr[...] = (g * u).astype(BF16)

    pending = down_runs[0] + down_runs[1]
    for n, (band0, bands, row0, rows) in enumerate(_DOWN_ORDER):
        needed = [run for run in pending if run.overlaps(band0, bands, row0, rows)]
        pending = [run for run in pending if run not in needed]
        with _scope(f'w_d{n}'):
            if needed:
                tail_stream.wait(*needed)
        w = wdt_v[pl.ds(band0, bands), pl.ds(row0, rows), :].reshape(bands * rows, wdt_v.shape[2])
        y = lax.dot_general(act_scr[...], w, _NT, preferred_element_type=F32)
        for i in range(bands):
            cols = pl.ds((band0 + i) * band_rows + row0, rows)
            part = 1.0 if _PURE else y[:, i * rows:(i + 1) * rows]
            out_v[:, cols] = (fin_scr[0, :, cols] + fin_scr[1, :, cols] * part).astype(out_v.dtype)
    assert not pending and tail_stream.pos == tail_stream.total

    store = pltpu.make_async_copy(out_v, out_hbm, new_sem())
    with _scope('out'):
        store.start()
        store.wait()


@jax.jit
def pallas_adaLN_cond__sliding_block_cached__moe_arch_mod__decode_kernel(
    A_x: jax.Array,
    A_k_cache: jax.Array,
    A_v_cache: jax.Array,
    A_wq: jax.Array,
    A_wo: jax.Array,
    B_x: jax.Array,
    B_w_r: jax.Array,
    B_w_gate: jax.Array,
    B_w_up: jax.Array,
    B_w_down: jax.Array,
    c: jax.Array,
    w_mod: jax.Array,
):
    del B_x
    batch, q_len, d_model = A_x.shape
    _, kv_heads, seq, head_dim = A_k_cache.shape
    window = min(4096, max(256, seq // 4))
    assert q_len == 1 and A_wq.shape[1] == 2 * kv_heads * head_dim

    wq, wot, wg, wu, wdt, wmod = (
        w.reshape(_BANDS, d_model // _BANDS, w.shape[1])
        for w in (A_wq, A_wo.T, B_w_gate, B_w_up, B_w_down.T, w_mod)
    )
    hbm = pl.BlockSpec(memory_space=pltpu.HBM)
    out = pl.pallas_call(
        _block_kernel,
        out_shape=jax.ShapeDtypeStruct((batch, d_model), A_x.dtype),
        in_specs=[hbm] * 11,
        out_specs=hbm,
        scratch_shapes=[
            pltpu.VMEM((2, _GROUP, window, head_dim), A_k_cache.dtype),
            pltpu.VMEM((2, _GROUP, window, head_dim), A_v_cache.dtype),
            *(pltpu.VMEM(w.shape, w.dtype) for w in (wq, wot, wg, wu, wdt, wmod)),
            pltpu.VMEM((batch, d_model), A_x.dtype),
            pltpu.VMEM(c.shape, c.dtype),
            pltpu.VMEM(B_w_r.shape, B_w_r.dtype),
            pltpu.VMEM((kv_heads, 2 * batch, head_dim), BF16),
            pltpu.VMEM((kv_heads, 2 * batch, head_dim), F32),
            pltpu.VMEM((batch, B_w_gate.shape[1]), BF16),
            pltpu.VMEM((2, batch, d_model), F32),
            pltpu.VMEM((batch, d_model), A_x.dtype),
            pltpu.SemaphoreType.DMA((16 + sum(len(lane) for lane in _DOWN_RUNS),)),
        ],
        compiler_params=pltpu.CompilerParams(
            vmem_limit_bytes=80 * 1024 * 1024,
            disable_bounds_checks=True,
            disable_semaphore_checks=True,
        ),
    )(A_x.reshape(batch, d_model), A_k_cache, A_v_cache, wq, wot, B_w_r, wg, wu, wdt, c, wmod)
    return out.reshape(A_x.shape)
```

```python
import jax
import jax.numpy as jnp
from jax import lax
import jax.experimental.pallas as pl
import jax.experimental.pallas.tpu as pltpu

F32 = jnp.float32
BF16 = jnp.bfloat16
_NT = (((1,), (1,)), ((), ()))

_TILE_ROWS = 8
_LANES = 128
_GROUP = 8
_SLAB = 64
_SPAN = 2
_LEAD = 56
_BANDS = 6
_TILES = {'mod': (5,), 'q': (6,), 'o': (6,), 'gu': (2, 3), 'd': (6,)}
_ORDER = 'bh'
_GU_SPAN = None
_PURE = False
_SCOPES = False
_DOWN_RUNS = (
    ((0, 3, 32, 64, (6,)), (0, 3, 0, 16, (6,)), (0, 3, 16, 16, (6,))),
    ((3, 3, 32, 32, (6,)), (3, 3, 64, 16, (6,)), (3, 3, 80, 16, (6,)),
     (3, 1, 0, 32, (18,)), (5, 1, 0, 32, (18,)), (4, 1, 0, 32, (18,))),
)
_DOWN_ORDER = (
    (0, 3, 32, 64), (3, 3, 32, 32), (0, 3, 0, 16), (3, 3, 64, 16), (0, 3, 16, 16), (3, 3, 80, 16),
    (3, 1, 0, 32), (5, 1, 0, 32), (4, 1, 0, 32),
)


def _scope(name):
    import contextlib
    return jax.named_scope(name) if _SCOPES else contextlib.nullcontext()


def _layernorm(x, eps=1e-5):
    d = x - jnp.mean(x, axis=-1, keepdims=True)
    v = jnp.mean(d * d, axis=-1, keepdims=True)
    return d / jnp.sqrt(v + eps)


class _Run:
    def __init__(self, src, dst, sem, band0, bands, row0, rows, tiles, span=None):
        self.src, self.dst, self.sem = src, dst, sem
        self.band0, self.bands, self.row0, self.rows = band0, bands, row0, rows
        cols, col = [], 0
        while col < src.shape[2]:
            width = min(tiles[len(cols) % len(tiles)] * _LANES, src.shape[2] - col)
            cols.append(pl.ds(col, width))
            col += width
        self.pieces = [
            (self, (pl.ds(band, span or bands), pl.ds(row, _TILE_ROWS), c))
            for row in range(row0, row0 + rows, _TILE_ROWS) for c in cols
            for band in range(band0, band0 + bands, span or bands)
        ]

    def overlaps(self, band0, bands, row0, rows):
        return (self.band0 < band0 + bands and band0 < self.band0 + self.bands
                and self.row0 < row0 + rows and row0 < self.row0 + self.rows)

    def wait(self):
        filled = self.dst.at[pl.ds(self.band0, self.bands), pl.ds(self.row0, self.rows)]
        pltpu.make_async_copy(filled, filled, self.sem).wait()


class _Stream:
    def __init__(self, *lanes):
        self.lanes = [[piece for run in lane for piece in run.pieces] for lane in lanes]
        self.total = max(len(lane) for lane in self.lanes)
        self.pos = 0

    def advance_to(self, pos):
        lo, hi = self.pos, min(pos, self.total)
        if hi <= lo:
            return
        cuts = (lo, (lo + hi + 1) // 2, hi)

        @pl.loop(0, 2)
        def _(part):
            for i in range(2):
                @pl.when(part == i)
                def _():
                    for n in range(cuts[i], cuts[i + 1]):
                        for queue, lane in enumerate(self.lanes):
                            if n < len(lane):
                                run, idx = lane[n]
                                pltpu.make_async_copy(
                                    run.src.at[idx], run.dst.at[idx], run.sem).start(priority=queue)

        self.pos = hi

    def wait(self, *runs):
        end = max(n + 1 for lane in self.lanes for n, (run, _) in enumerate(lane) if run in runs)
        with _scope('issue'):
            self.advance_to(end + _LEAD)
        for run in runs:
            with _scope('wait'):
                run.wait()


def _block_kernel(
    x_hbm, k_hbm, v_hbm, wq_hbm, wot_hbm, wr_hbm, wg_hbm, wu_hbm, wdt_hbm, c_hbm, wmod_hbm,
    out_hbm,
    k_buf, v_buf, wq_v, wot_v, wg_v, wu_v, wdt_v, wmod_v, x_v, c_v, wr_v,
    q_scr, o_scr, act_scr, fin_scr, out_v,
    sems,
):
    spare = iter(range(4, sems.shape[0]))

    def new_sem():
        return sems.at[next(spare)]

    batch, kv_heads, seq, head_dim = k_hbm.shape
    window = k_buf.shape[2]
    d_model = x_v.shape[1]
    band_rows = d_model // _BANDS
    per_batch = kv_heads // _GROUP
    n_groups = batch * per_batch
    spans = _GROUP // _SPAN
    slabs = window // _SLAB * spans
    slabs_per_head = (slabs - _LEAD) // _GROUP
    assert _LEAD + _GROUP * slabs_per_head == slabs

    def locate(group, j):
        if _ORDER == 'bh':
            b, part = group // per_batch, group % per_batch
        else:
            b, part = group % batch, group // batch
        return b, (j // _SPAN * per_batch + part) * _SPAN + j % _SPAN

    def start_kv(group, lo, hi):
        @pl.loop(lo, hi)
        def _(n):
            row = pl.multiple_of(n // spans * _SLAB, _SLAB)
            j = n % spans * _SPAN
            b, head = locate(group, j)
            for queue, (src, dst) in enumerate(((k_hbm, k_buf), (v_hbm, v_buf))):
                pltpu.make_async_copy(
                    src.at[b, pl.ds(head, _SPAN), pl.ds(seq - window + row, _SLAB), :],
                    dst.at[group % 2, pl.ds(j, _SPAN), pl.ds(row, _SLAB), :],
                    sems.at[2 * queue + group % 2],
                ).start(priority=queue)

    def wait_kv(group):
        for queue, buf in enumerate((k_buf, v_buf)):
            filled = buf.at[group % 2]
            pltpu.make_async_copy(filled, filled, sems.at[2 * queue + group % 2]).wait()

    def halves(src, dst, n, tiles):
        half = _BANDS // 2
        return [_Run(src, dst, new_sem(), q * half, half, 0, band_rows, tiles) for q in range(2)]

    def matrix(ref):
        return ref[...].reshape(d_model, ref.shape[2])

    mod_runs = halves(wmod_hbm, wmod_v, 0, _TILES['mod'])
    q_runs = halves(wq_hbm, wq_v, 1, _TILES['q'])
    o_runs = halves(wot_hbm, wot_v, 2, _TILES['o'])
    gu_runs = [
        _Run(src, dst, new_sem(), 0, _BANDS, 0, band_rows, _TILES['gu'], _GU_SPAN)
        for q, (src, dst) in enumerate(((wg_hbm, wg_v), (wu_hbm, wu_v)))
    ]
    down_runs = [
        [_Run(wdt_hbm, wdt_v, new_sem(), *spec) for n, spec in enumerate(lane)]
        for q, lane in enumerate(_DOWN_RUNS)
    ]
    head_stream = _Stream(*zip(mod_runs, q_runs))
    tail_stream = _Stream(*([o_runs[q], gu_runs[q]] + down_runs[q] for q in range(2)))

    small = [
        pltpu.make_async_copy(src, dst, new_sem())
        for n, (src, dst) in enumerate(((c_hbm, c_v), (x_hbm, x_v), (wr_hbm, wr_v)))
    ]
    head_stream.advance_to(4)
    for copy in small:
        copy.start()
    with _scope('w_mod'):
        head_stream.wait(*mod_runs)
    for copy in small:
        copy.wait()
    cond = jax.nn.silu(c_v[...].astype(F32)).astype(BF16)
    mod = jnp.dot(cond, matrix(wmod_v), preferred_element_type=F32)
    shift_a, scale_a, gate_a, shift_b, scale_b, gate_b = (
        mod[:, n * d_model:(n + 1) * d_model] for n in range(6)
    )
    x0 = x_v[...].astype(F32)
    h1 = (_layernorm(x0) * (1.0 + scale_a) + shift_a).astype(BF16)
    o_scr[...] = jnp.zeros(o_scr.shape, F32)

    with _scope('w_q'):
        head_stream.advance_to(head_stream.total)
        start_kv(0, 0, _LEAD)
        head_stream.wait(*q_runs)
    q = jnp.dot(h1, matrix(wq_v), preferred_element_type=F32)
    for head in range(kv_heads):
        pair = [q[:, (2 * head + r) * head_dim:(2 * head + r + 1) * head_dim] for r in range(2)]
        q_scr[head] = jnp.concatenate(pair, axis=0).astype(BF16)
    with _scope('i_kv0'):
        start_kv(0, _LEAD, slabs)

    row_batch = lax.broadcasted_iota(jnp.int32, (2 * batch, head_dim), 0) % batch

    def attend(group, j):
        if _PURE in (True, 'attn'):
            return
        b, head = locate(group, j)
        s = lax.dot_general(q_scr[head], k_buf[group % 2, j], _NT, preferred_element_type=F32)
        s = s * head_dim ** -0.5
        p = jnp.exp(s - jnp.max(s, axis=-1, keepdims=True))
        denom = jnp.sum(p, axis=-1, keepdims=True)
        o = jnp.dot(p.astype(BF16), v_buf[group % 2, j], preferred_element_type=F32) / denom
        o_scr[head] = jnp.where(row_batch == b, o, o_scr[head])

    with _scope('main'):
        @pl.loop(0, n_groups - 1)
        def _(group):
            start_kv(group + 1, 0, _LEAD)
            wait_kv(group)

            @pl.loop(0, _GROUP)
            def _(j):
                attend(group, j)
                lo = _LEAD + j * slabs_per_head
                start_kv(group + 1, lo, lo + slabs_per_head)

    with _scope('last'):
        tail_stream.advance_to(_LEAD)
        wait_kv(n_groups - 1)
        for j in range(0, _GROUP, 2):
            pl.loop(j, j + 2)(lambda jj: attend(n_groups - 1, jj))
            tail_stream.advance_to(_LEAD + (j + 2) * slabs_per_head)

    with _scope('w_o'):
        tail_stream.wait(*o_runs)
    attn = jnp.concatenate(
        [o_scr[head, pl.ds(r * batch, batch), :] for head in range(kv_heads) for r in range(2)],
        axis=1,
    ).astype(BF16)
    x1 = x0 + gate_a * lax.dot_general(attn, matrix(wot_v), _NT, preferred_element_type=F32)
    h2 = _layernorm(x1) * (1.0 + scale_b) + shift_b
    h2_mxu = h2.astype(BF16)
    w_r = wr_v[...].astype(F32).reshape(1, d_model)
    route = jax.nn.sigmoid(jnp.sum(h2_mxu.astype(F32) * w_r, axis=-1, keepdims=True))
    fin_scr[0] = x1 + gate_b * (h2 + h2 * 0.0)
    fin_scr[1] = gate_b * route

    with _scope('w_gu'):
        tail_stream.wait(*gu_runs)
    g = jax.nn.silu(jnp.dot(h2_mxu, matrix(wg_v), preferred_element_type=F32))
    u = jnp.dot(h2_mxu, matrix(wu_v), preferred_element_type=F32)
    act_scr[...] = (g * u).astype(BF16)

    pending = down_runs[0] + down_runs[1]
    for n, (band0, bands, row0, rows) in enumerate(_DOWN_ORDER):
        needed = [run for run in pending if run.overlaps(band0, bands, row0, rows)]
        pending = [run for run in pending if run not in needed]
        with _scope(f'w_d{n}'):
            if needed:
                tail_stream.wait(*needed)
        w = wdt_v[pl.ds(band0, bands), pl.ds(row0, rows), :].reshape(bands * rows, wdt_v.shape[2])
        y = lax.dot_general(act_scr[...], w, _NT, preferred_element_type=F32)
        for i in range(bands):
            cols = pl.ds((band0 + i) * band_rows + row0, rows)
            part = 1.0 if _PURE in (True, 'down') else y[:, i * rows:(i + 1) * rows]
            out_v[:, cols] = (fin_scr[0, :, cols] + fin_scr[1, :, cols] * part).astype(out_v.dtype)
    assert not pending and tail_stream.pos == tail_stream.total

    store = pltpu.make_async_copy(out_v, out_hbm, new_sem())
    with _scope('out'):
        store.start()
        store.wait()


@jax.jit
def pallas_adaLN_cond__sliding_block_cached__moe_arch_mod__decode_kernel(
    A_x: jax.Array,
    A_k_cache: jax.Array,
    A_v_cache: jax.Array,
    A_wq: jax.Array,
    A_wo: jax.Array,
    B_x: jax.Array,
    B_w_r: jax.Array,
    B_w_gate: jax.Array,
    B_w_up: jax.Array,
    B_w_down: jax.Array,
    c: jax.Array,
    w_mod: jax.Array,
):
    del B_x
    batch, q_len, d_model = A_x.shape
    _, kv_heads, seq, head_dim = A_k_cache.shape
    window = min(4096, max(256, seq // 4))
    assert q_len == 1 and A_wq.shape[1] == 2 * kv_heads * head_dim

    wq, wot, wg, wu, wdt, wmod = (
        w.reshape(_BANDS, d_model // _BANDS, w.shape[1])
        for w in (A_wq, A_wo.T, B_w_gate, B_w_up, B_w_down.T, w_mod)
    )
    hbm = pl.BlockSpec(memory_space=pltpu.HBM)
    out = pl.pallas_call(
        _block_kernel,
        out_shape=jax.ShapeDtypeStruct((batch, d_model), A_x.dtype),
        in_specs=[hbm] * 11,
        out_specs=hbm,
        scratch_shapes=[
            pltpu.VMEM((2, _GROUP, window, head_dim), A_k_cache.dtype),
            pltpu.VMEM((2, _GROUP, window, head_dim), A_v_cache.dtype),
            *(pltpu.VMEM(w.shape, w.dtype) for w in (wq, wot, wg, wu, wdt, wmod)),
            pltpu.VMEM((batch, d_model), A_x.dtype),
            pltpu.VMEM(c.shape, c.dtype),
            pltpu.VMEM(B_w_r.shape, B_w_r.dtype),
            pltpu.VMEM((kv_heads, 2 * batch, head_dim), BF16),
            pltpu.VMEM((kv_heads, 2 * batch, head_dim), F32),
            pltpu.VMEM((batch, B_w_gate.shape[1]), BF16),
            pltpu.VMEM((2, batch, d_model), F32),
            pltpu.VMEM((batch, d_model), A_x.dtype),
            pltpu.SemaphoreType.DMA((16 + sum(len(lane) for lane in _DOWN_RUNS),)),
        ],
        compiler_params=pltpu.CompilerParams(
            vmem_limit_bytes=80 * 1024 * 1024,
            disable_bounds_checks=True,
            disable_semaphore_checks=True,
        ),
    )(A_x.reshape(batch, d_model), A_k_cache, A_v_cache, wq, wot, B_w_r, wg, wu, wdt, c, wmod)
    return out.reshape(A_x.shape)
```

```python
import jax
import jax.numpy as jnp
from jax import lax
import jax.experimental.pallas as pl
import jax.experimental.pallas.tpu as pltpu

F32 = jnp.float32
BF16 = jnp.bfloat16
_NT = (((1,), (1,)), ((), ()))

_TILE_ROWS = 8
_LANES = 128
_LEAD = 56
_GROUP = 8
_SPAN = 2
_SLAB = 64
_BANDS = 6
_DOWN_FETCH = (
    ((0, 3, 32, 64), (0, 3, 0, 16), (0, 3, 16, 16)),
    ((3, 3, 32, 32), (3, 3, 64, 16), (3, 3, 80, 16), (3, 1, 0, 32), (5, 1, 0, 32), (4, 1, 0, 32)),
)
_DOWN_USE = (
    (0, 3, 32, 64), (3, 3, 32, 32), (0, 3, 0, 16), (3, 3, 64, 16), (0, 3, 16, 16), (3, 3, 80, 16),
    (3, 1, 0, 32), (5, 1, 0, 32), (4, 1, 0, 32),
)
_NUM_SEMS = 4 + 6 + len(_DOWN_USE) + 4


def _layernorm(x, eps=1e-5):
    d = x - jnp.mean(x, axis=-1, keepdims=True)
    v = jnp.mean(d * d, axis=-1, keepdims=True)
    return d / jnp.sqrt(v + eps)


class _Block:
    def __init__(self, src, dst, sem, band0, bands, row0, rows, span, tiles):
        self.src, self.dst, self.sem = src, dst, sem
        self.where = (pl.ds(band0, bands), pl.ds(row0, rows))
        width = src.shape[2] // _LANES
        self.pieces = []
        for row in range(row0, row0 + rows, _TILE_ROWS):
            first = -(row // _TILE_ROWS) * width % tiles
            cuts = [0, *range(first or tiles, width, tiles), width]
            self.pieces += [
                (pl.ds(band, span), pl.ds(row, _TILE_ROWS), pl.ds(lo * _LANES, (hi - lo) * _LANES))
                for lo, hi in zip(cuts[:-1], cuts[1:])
                for band in range(band0, band0 + bands, span)
            ]

    def start(self, piece, queue):
        pltpu.make_async_copy(self.src.at[piece], self.dst.at[piece], self.sem).start(priority=queue)

    def wait(self):
        filled = self.dst.at[self.where]
        pltpu.make_async_copy(filled, filled, self.sem).wait()


class _Stream:
    def __init__(self, *lanes):
        self.lanes = [[(block, piece) for block in lane for piece in block.pieces] for lane in lanes]
        self.total = max(len(lane) for lane in self.lanes)
        self.pos = 0

    def advance_to(self, pos):
        lo, hi = self.pos, min(pos, self.total)
        if hi <= lo:
            return
        cuts = (lo, (lo + hi) // 2, hi)

        def start(part):
            for n in range(cuts[part], cuts[part + 1]):
                for queue, lane in enumerate(self.lanes):
                    if n < len(lane):
                        block, piece = lane[n]
                        block.start(piece, queue)

        @pl.loop(0, 2)
        def _(part):
            pl.when(part == 0)(lambda: start(0))
            pl.when(part == 1)(lambda: start(1))

        self.pos = hi

    def wait(self, *blocks):
        end = max(n + 1 for lane in self.lanes for n, (b, _) in enumerate(lane) if b in blocks)
        self.advance_to(end + _LEAD)
        for block in blocks:
            block.wait()


def _block_kernel(
    x_hbm, k_hbm, v_hbm, wq_hbm, wot_hbm, wr_hbm, wg_hbm, wu_hbm, wdt_hbm, c_hbm, wmod_hbm,
    out_hbm,
    k_buf, v_buf, wq_v, wot_v, wg_v, wu_v, wdt_v, wmod_v, x_v, c_v, wr_v,
    q_scr, o_scr, act_scr, fin_scr, out_v,
    sems,
):
    batch, kv_heads, seq, head_dim = k_hbm.shape
    window = k_buf.shape[2]
    d_model = x_v.shape[1]
    band_rows = d_model // _BANDS
    spare_sems = iter(range(4, _NUM_SEMS))

    def new_sem():
        return sems.at[next(spare_sems)]

    groups_per_row = kv_heads // _GROUP
    n_groups = batch * groups_per_row
    spans = _GROUP // _SPAN
    kv_copies = window // _SLAB * spans
    copies_per_head = (kv_copies - _LEAD) // _GROUP
    assert _LEAD + _GROUP * copies_per_head == kv_copies

    def locate(group, j):
        part = group % groups_per_row
        return group // groups_per_row, (j // _SPAN * groups_per_row + part) * _SPAN + j % _SPAN

    def start_kv(group, lo, hi):
        @pl.loop(lo, hi)
        def _(n):
            row = pl.multiple_of(n // spans * _SLAB, _SLAB)
            j = n % spans * _SPAN
            b, head = locate(group, j)
            for queue, (src, dst) in enumerate(((k_hbm, k_buf), (v_hbm, v_buf))):
                pltpu.make_async_copy(
                    src.at[b, pl.ds(head, _SPAN), pl.ds(seq - window + row, _SLAB), :],
                    dst.at[group % 2, pl.ds(j, _SPAN), pl.ds(row, _SLAB), :],
                    sems.at[2 * queue + group % 2],
                ).start(priority=queue)

    def wait_kv(group):
        for queue, buf in enumerate((k_buf, v_buf)):
            filled = buf.at[group % 2]
            pltpu.make_async_copy(filled, filled, sems.at[2 * queue + group % 2]).wait()

    def side_by_side(*pairs):
        return [_Block(src, dst, new_sem(), 0, _BANDS, 0, band_rows, 2, 8) for src, dst in pairs]

    def matrix(ref):
        return ref[...].reshape(d_model, ref.shape[2])

    half = _BANDS // 2
    mod_blocks = [
        _Block(wmod_hbm, wmod_v, new_sem(), q * half, half, 0, band_rows, half, 5) for q in range(2)
    ]
    qo_blocks = side_by_side((wq_hbm, wq_v), (wot_hbm, wot_v))
    gu_blocks = side_by_side((wg_hbm, wg_v), (wu_hbm, wu_v))
    down_blocks = {
        where: _Block(wdt_hbm, wdt_v, new_sem(), *where, where[1], 8 if where[1] > 1 else 18)
        for where in _DOWN_USE
    }
    head_stream = _Stream(*zip(mod_blocks, qo_blocks))
    tail_stream = _Stream(
        *([gu_blocks[q]] + [down_blocks[where] for where in _DOWN_FETCH[q]] for q in range(2))
    )

    small = [
        pltpu.make_async_copy(src, dst, new_sem())
        for src, dst in ((c_hbm, c_v), (x_hbm, x_v), (wr_hbm, wr_v))
    ]
    head_stream.advance_to(4)
    for copy in small:
        copy.start()
    head_stream.wait(*mod_blocks)
    for copy in small:
        copy.wait()
    cond = jax.nn.silu(c_v[...].astype(F32)).astype(BF16)
    mod = jnp.dot(cond, matrix(wmod_v), preferred_element_type=F32)
    shift_a, scale_a, gate_a, shift_b, scale_b, gate_b = (
        mod[:, n * d_model:(n + 1) * d_model] for n in range(6)
    )
    x0 = x_v[...].astype(F32)
    h1 = (_layernorm(x0) * (1.0 + scale_a) + shift_a).astype(BF16)
    o_scr[...] = jnp.zeros(o_scr.shape, F32)

    head_stream.advance_to(head_stream.total)
    start_kv(0, 0, _LEAD)
    head_stream.wait(*qo_blocks)
    q = jnp.dot(h1, matrix(wq_v), preferred_element_type=F32)
    for head in range(kv_heads):
        pair = [q[:, (2 * head + r) * head_dim:(2 * head + r + 1) * head_dim] for r in range(2)]
        q_scr[head] = jnp.concatenate(pair, axis=0).astype(BF16)
    start_kv(0, _LEAD, kv_copies)

    row_batch = lax.broadcasted_iota(jnp.int32, (2 * batch, head_dim), 0) % batch

    def attend(group, j):
        b, head = locate(group, j)
        s = lax.dot_general(q_scr[head], k_buf[group % 2, j], _NT, preferred_element_type=F32)
        s = s * head_dim ** -0.5
        p = jnp.exp(s - jnp.max(s, axis=-1, keepdims=True))
        denom = jnp.sum(p, axis=-1, keepdims=True)
        o = jnp.dot(p.astype(BF16), v_buf[group % 2, j], preferred_element_type=F32) / denom
        o_scr[head] = jnp.where(row_batch == b, o, o_scr[head])

    @pl.loop(0, n_groups - 1)
    def _(group):
        start_kv(group + 1, 0, _LEAD)
        wait_kv(group)

        @pl.loop(0, _GROUP)
        def _(j):
            attend(group, j)
            lo = _LEAD + j * copies_per_head
            start_kv(group + 1, lo, lo + copies_per_head)

    tail_stream.advance_to(_LEAD)
    wait_kv(n_groups - 1)
    for j0 in range(0, _GROUP, 2):
        pl.loop(j0, j0 + 2)(lambda j: attend(n_groups - 1, j))
        tail_stream.advance_to(_LEAD + (j0 + 2) * copies_per_head)

    attn = jnp.concatenate(
        [o_scr[head, pl.ds(r * batch, batch), :] for head in range(kv_heads) for r in range(2)],
        axis=1,
    ).astype(BF16)
    x1 = x0 + gate_a * lax.dot_general(attn, matrix(wot_v), _NT, preferred_element_type=F32)
    h2 = _layernorm(x1) * (1.0 + scale_b) + shift_b
    h2_mxu = h2.astype(BF16)
    w_r = wr_v[...].astype(F32).reshape(1, d_model)
    route = jax.nn.sigmoid(jnp.sum(h2_mxu.astype(F32) * w_r, axis=-1, keepdims=True))
    fin_scr[0] = x1 + gate_b * (h2 + h2 * 0.0)
    fin_scr[1] = gate_b * route

    tail_stream.wait(*gu_blocks)
    g = jax.nn.silu(jnp.dot(h2_mxu, matrix(wg_v), preferred_element_type=F32))
    u = jnp.dot(h2_mxu, matrix(wu_v), preferred_element_type=F32)
    act_scr[...] = (g * u).astype(BF16)

    for where in _DOWN_USE:
        band0, bands, row0, rows = where
        tail_stream.wait(down_blocks[where])
        w = wdt_v[pl.ds(band0, bands), pl.ds(row0, rows), :].reshape(bands * rows, wdt_v.shape[2])
        y = lax.dot_general(act_scr[...], w, _NT, preferred_element_type=F32)
        for i in range(bands):
            cols = pl.ds((band0 + i) * band_rows + row0, rows)
            out = fin_scr[0, :, cols] + fin_scr[1, :, cols] * y[:, i * rows:(i + 1) * rows]
            out_v[:, cols] = out.astype(out_v.dtype)

    store = pltpu.make_async_copy(out_v, out_hbm, new_sem())
    store.start()
    store.wait()


@jax.jit
def pallas_adaLN_cond__sliding_block_cached__moe_arch_mod__decode_kernel(
    A_x: jax.Array,
    A_k_cache: jax.Array,
    A_v_cache: jax.Array,
    A_wq: jax.Array,
    A_wo: jax.Array,
    B_x: jax.Array,
    B_w_r: jax.Array,
    B_w_gate: jax.Array,
    B_w_up: jax.Array,
    B_w_down: jax.Array,
    c: jax.Array,
    w_mod: jax.Array,
):
    del B_x
    batch, q_len, d_model = A_x.shape
    _, kv_heads, seq, head_dim = A_k_cache.shape
    window = min(4096, max(256, seq // 4))
    assert q_len == 1 and A_wq.shape[1] == 2 * kv_heads * head_dim
    assert d_model == sum(bands * rows for _, bands, _, rows in _DOWN_USE)

    wq, wot, wg, wu, wdt, wmod = (
        w.reshape(_BANDS, d_model // _BANDS, w.shape[1])
        for w in (A_wq, A_wo.T, B_w_gate, B_w_up, B_w_down.T, w_mod)
    )
    hbm = pl.BlockSpec(memory_space=pltpu.HBM)
    out = pl.pallas_call(
        _block_kernel,
        out_shape=jax.ShapeDtypeStruct((batch, d_model), A_x.dtype),
        in_specs=[hbm] * 11,
        out_specs=hbm,
        scratch_shapes=[
            pltpu.VMEM((2, _GROUP, window, head_dim), A_k_cache.dtype),
            pltpu.VMEM((2, _GROUP, window, head_dim), A_v_cache.dtype),
            *(pltpu.VMEM(w.shape, w.dtype) for w in (wq, wot, wg, wu, wdt, wmod)),
            pltpu.VMEM((batch, d_model), A_x.dtype),
            pltpu.VMEM(c.shape, c.dtype),
            pltpu.VMEM(B_w_r.shape, B_w_r.dtype),
            pltpu.VMEM((kv_heads, 2 * batch, head_dim), BF16),
            pltpu.VMEM((kv_heads, 2 * batch, head_dim), F32),
            pltpu.VMEM((batch, B_w_gate.shape[1]), BF16),
            pltpu.VMEM((2, batch, d_model), F32),
            pltpu.VMEM((batch, d_model), A_x.dtype),
            pltpu.SemaphoreType.DMA((_NUM_SEMS,)),
        ],
        compiler_params=pltpu.CompilerParams(
            vmem_limit_bytes=80 * 1024 * 1024,
            disable_bounds_checks=True,
            disable_semaphore_checks=True,
        ),
    )(A_x.reshape(batch, d_model), A_k_cache, A_v_cache, wq, wot, B_w_r, wg, wu, wdt, c, wmod)
    return out.reshape(A_x.shape)
```
